```python
import os as _os
_os.environ.setdefault('JAX_PLATFORMS', 'cpu')
import jax
import jax.numpy as jnp

def _softmax(x, axis=-1):
    return jax.nn.softmax(x, axis=axis)

def _gelu(x):
    return jax.nn.gelu(x, approximate=True)

def _silu(x):
    return jax.nn.silu(x)

def _sigmoid(x):
    return jax.nn.sigmoid(x)

def _layernorm(x, axis=-1, eps=1e-05):
    m = jnp.mean(x, axis=axis, keepdims=True)
    v = jnp.var(x, axis=axis, keepdims=True)
    return (x - m) / jnp.sqrt(v + eps)

def _scatter_add(tgt, idx, src, axis=0):
    return tgt.at[idx].add(src)

def _segment_sum(src, seg, n):
    return jax.ops.segment_sum(src, seg, n)

class _Rng:

    def __init__(self, key):
        self._k = key

    def _next(self):
        self._k, sub = jax.random.split(self._k)
        return sub

    def normal(self, shape):
        return jax.random.normal(self._next(), shape, dtype=jnp.bfloat16)

    def randint(self, lo, hi, shape):
        return jax.random.randint(self._next(), shape, lo, hi, dtype=jnp.int32)

    def uniform(self, shape, lo=0.0, hi=1.0):
        return jax.random.uniform(self._next(), shape, jnp.bfloat16, lo, hi)

    def permutation(self, n):
        return jax.random.permutation(self._next(), n)
kernel_name = 'adaLN_cond__sliding_local_dilated__dense_activation_silu__prompt'

def setup_inputs():
    _rng = _Rng(jax.random.key(int.from_bytes(__import__("os").urandom(4), "little")))
    _w = lambda a: (lambda t: t.astype(jnp.bfloat16) if jnp.issubdtype(t.dtype, jnp.floating) else t)(jnp.asarray(a))

    def _A_setup():
        B, S, D = (1, 2048, 512)
        return {'x': _w((lambda *s: _rng.normal(s) * 0.05)(B, S, D)), 'wqkv': _w((lambda *s: _rng.normal(s) * 0.05)(D, 3 * D)), 'wo': _w((lambda *s: _rng.normal(s) * 0.05)(D, D))}
    _A_in = _A_setup()

    def _B_setup():
        B, S, D, F = (1, 2048, 512, 1792)
        return {'x': _w((lambda *s: _rng.normal(s) * 0.05)(B, S, D)), 'w1': _w((lambda *s: _rng.normal(s) * 0.8)(D, F) * D ** (-0.5)), 'w2': _w((lambda *s: _rng.normal(s) * 0.8)(F, D) * F ** (-0.5))}
    _B_in = _B_setup()
    return {'A_x': _A_in['x'], 'A_wqkv': _A_in['wqkv'], 'A_wo': _A_in['wo'], 'B_x': _B_in['x'], 'B_w1': _B_in['w1'], 'B_w2': _B_in['w2'], 'c': _w((lambda *s: _rng.normal(s) * 0.05)(1, 512) * 8.0), 'w_mod': _w((lambda *s: _rng.normal(s) * 0.05)(512, 6 * 512) * 512 ** (-0.5) * 8.0)}

def reference(A_x, A_wqkv, A_wo, B_x, B_w1, B_w2, c, w_mod):

    def _A_ref(x, wqkv, wo):
        B, S, D = x.shape
        H = 32
        Dh = D // H
        W, dil = (8, 2)
        qkv = (lambda x, *d: x.transpose(*d))((x @ wqkv).reshape(B, S, 3, H, Dh), 2, 0, 3, 1, 4)
        q, k, v = (qkv[0], qkv[1], qkv[2])
        scale = Dh ** (-0.5)
        pos = jnp.arange(S)
        off = jnp.arange(W) * dil
        idx = pos[:, None] - off[None, :]
        mask = idx >= 0
        idx_c = jnp.where(mask, idx, 0).reshape(-1)
        kg = k[:, :, idx_c, :].reshape(B, H, S, W, Dh)
        vg = v[:, :, idx_c, :].reshape(B, H, S, W, Dh)
        logits = jnp.einsum('bhsd,bhswd->bhsw', q, kg) * scale
        logits = jnp.where(mask[None, None, :, :], logits, -1000000000.0)
        attn = _softmax(logits, axis=-1)
        o = jnp.einsum('bhsw,bhswd->bhsd', attn, vg)
        return (lambda x, *d: x.transpose(*d))(o, 0, 2, 1, 3).reshape(B, S, D) @ wo

    def _B_ref(x, w1, w2):
        h = jnp.einsum('bsd,df->bsf', x, w1)
        h = _silu(h)
        out = jnp.einsum('bsf,fd->bsd', h, w2)
        return out
    x = A_x
    mod = (_silu(c) @ w_mod).reshape(c.shape[0], 6, 1, -1)
    sa, ca, ga, sb, cb, gb = (mod[:, 0].copy(), mod[:, 1].copy(), mod[:, 2].copy(), mod[:, 3].copy(), mod[:, 4].copy(), mod[:, 5].copy())
    h = _layernorm(x, axis=-1) * (1 + ca) + sa
    x = x + ga * _A_ref(h, A_wqkv, A_wo)
    h = _layernorm(x, axis=-1) * (1 + cb) + sb
    x = x + gb * _B_ref(h, B_w1, B_w2)
    return x
```

```python
import functools
import jax
import jax.numpy as jnp
from jax import lax
import jax.experimental.pallas as pl
import jax.experimental.pallas.tpu as pltpu

S, D, F = 2048, 512, 1792
H, DH, W, DIL = 32, 16, 8, 2
TM = 256
NB = S // TM
HALO = 16
CH = 16
NC = D // 128
LOG2E = 1.4426950408889634
EPS = 1e-5
FC = 256
GOFF = 0.0
GSPAN = 0.93
QSCALE = DH ** -0.5 * LOG2E
F32 = jnp.float32
BF16 = jnp.bfloat16


def _dot(a, b):
    return jnp.dot(a, b, preferred_element_type=F32)


def _ln(x):
    m = jnp.sum(x, axis=-1, keepdims=True) * (1.0 / D)
    xc = x - m
    v = jnp.sum(xc * xc, axis=-1, keepdims=True) * (1.0 / D)
    return xc * lax.rsqrt(v + EPS)


def _kernel(x_hbm, wqkv_hbm, wo_hbm, w1_hbm, w2_hbm, c_ref, wmod_hbm, out_hbm,
            x_v, wqkv_v, wqkv_p, wo_v, wo_p, w1_v, w2_v, wmod_v, out_v,
            q_s, k_s, v_s, o_s, mod_s, zero_s, sem_w, sem_x, sem_o):

    def x_copy(i):
        return pltpu.make_async_copy(x_hbm.at[0, pl.ds(i * TM, TM), :],
                                     x_v.at[pl.ds(i * TM, TM), :], sem_x.at[i])

    def o_copy(i):
        return pltpu.make_async_copy(out_v.at[pl.ds(i * TM, TM), :],
                                     out_hbm.at[0, pl.ds(i * TM, TM), :], sem_o.at[i])

    cp_qkv = pltpu.make_async_copy(wqkv_hbm, wqkv_v, sem_w.at[0])
    cp_m1 = pltpu.make_async_copy(wmod_hbm.at[:, pl.ds(0, 2 * D)], wmod_v.at[:, pl.ds(0, 2 * D)], sem_w.at[1])
    cp_m2 = pltpu.make_async_copy(wmod_hbm.at[:, pl.ds(2 * D, 4 * D)], wmod_v.at[:, pl.ds(2 * D, 4 * D)], sem_w.at[2])
    cp_wo = pltpu.make_async_copy(wo_hbm, wo_v, sem_w.at[3])
    cp_w1 = pltpu.make_async_copy(w1_hbm, w1_v, sem_w.at[4])
    cp_w2 = pltpu.make_async_copy(w2_hbm, w2_v, sem_w.at[5])

    cp_qkv.start()
    x_copy(0).start()
    cp_m1.start()
    cp_wo.start()
    cp_m2.start()
    x_copy(1).start()
    cp_w1.start()
    cp_w2.start()
    for i in range(2, NB):
        x_copy(i).start()

    r = lax.broadcasted_iota(jnp.int32, (D, D), 0)
    cidx = lax.broadcasted_iota(jnp.int32, (D, D), 1)
    P = jnp.where(r == (cidx % H) * DH + cidx // H, 1.0, 0.0).astype(BF16)
    Pt = jnp.where(cidx == (r % H) * DH + r // H, 1.0, 0.0).astype(BF16)

    cp_qkv.wait()
    for t in range(3):
        wqkv_p[:, t * D:(t + 1) * D] = _dot(wqkv_v[:, t * D:(t + 1) * D], P).astype(BF16)

    cf = c_ref[...].astype(F32)
    sc = (cf * jax.nn.sigmoid(cf)).astype(BF16)
    sc8 = jnp.broadcast_to(sc, (8, D))
    cp_m1.wait()
    mod_s[:, 0:2 * D] = _dot(sc8, wmod_v[:, 0:2 * D])

    zero_s[...] = jnp.zeros((CH, 128), jnp.int32)

    def row0(i):
        return i * TM if isinstance(i, int) else pl.multiple_of(i * TM, TM)

    def a_qkv(i):
        first = isinstance(i, int) and i == 0
        x = x_v[pl.ds(row0(i), TM), :].astype(F32)
        sa = mod_s[0:1, 0:D]
        ca = mod_s[0:1, D:2 * D]
        h = (_ln(x) * (1.0 + ca) + sa).astype(BF16)
        if not first:
            k_s[:, 0:HALO, :] = k_s[:, TM:TM + HALO, :]
            v_s[:, 0:HALO, :] = v_s[:, TM:TM + HALO, :]
        qkv = _dot(h, wqkv_p[...])
        q_s[...] = qkv[:, 0:D]
        for c in range(NC):
            k_s[c, HALO:HALO + TM, :] = qkv[:, D + c * 128:D + (c + 1) * 128]
            v_s[c, HALO:HALO + TM, :] = qkv[:, 2 * D + c * 128:2 * D + (c + 1) * 128]
        if first:
            for c in range(NC):
                k_s[c, 0:HALO, :] = jnp.broadcast_to(k_s[c, HALO:HALO + 1, :], (HALO, 128))
                v_s[c, 0:HALO, :] = jnp.broadcast_to(v_s[c, HALO:HALO + 1, :], (HALO, 128))

    def a_attn(first, ch_lo, ch_hi, gate=None):
        never = zero_s[...] != 0
        for ch in range(ch_lo, ch_hi):
            b = ch * CH
            if gate is None:
                qscale = QSCALE
            else:
                qscale = jnp.where(never, gate(ch), QSCALE)
            q = [q_s[b:b + CH, c * 128:(c + 1) * 128] * qscale for c in range(NC)]
            ls = []
            for w in range(W):
                o = HALO + b - DIL * w
                s = q[0] * k_s[0, o:o + CH, :]
                for c in range(1, NC):
                    s = s + q[c] * k_s[c, o:o + CH, :]
                s = s + pltpu.roll(s, 64, 1)
                s = s + pltpu.roll(s, 32, 1)
                if first and b < DIL * w:
                    pos = lax.broadcasted_iota(jnp.int32, (CH, 128), 0) + b
                    s = jnp.where(pos >= DIL * w, s, -1e9 * LOG2E)
                ls.append(s)
            m = ls[0]
            for w in range(1, W):
                m = jnp.maximum(m, ls[w])
            ps = [jnp.exp2(l - m) for l in ls]
            den = ps[0]
            for w in range(1, W):
                den = den + ps[w]
            inv = 1.0 / den
            for c in range(NC):
                acc = ps[0] * v_s[c, HALO + b:HALO + b + CH, :]
                for w in range(1, W):
                    o = HALO + b - DIL * w
                    acc = acc + ps[w] * v_s[c, o:o + CH, :]
                o_s[b:b + CH, c * 128:(c + 1) * 128] = (acc * inv).astype(BF16)

    def b_wo():
        return _dot(o_s[...], wo_p[...])

    def b_ln(i, att):
        ga = mod_s[0:1, 2 * D:3 * D]
        sb = mod_s[0:1, 3 * D:4 * D]
        cb = mod_s[0:1, 4 * D:5 * D]
        x1 = x_v[pl.ds(row0(i), TM), :].astype(F32) + ga * att
        h2 = (_ln(x1) * (0.5 + 0.5 * cb) + 0.5 * sb).astype(BF16)
        return x1, h2

    NF = F // FC

    def b_mlp(i, x1, h2):
        gb = mod_s[0:1, 5 * D:6 * D]
        seq = []
        ts = [None] * NF

        def w1c(k):
            ts[k] = _dot(h2, w1_v[:, k * FC:(k + 1) * FC])
            seq.append(ts[k])

        w1c(0)
        y = None
        for k in range(NF):
            if k + 1 < NF:
                w1c(k + 1)
            t = ts[k]
            g = (t + t * jnp.tanh(t)).astype(BF16)
            p = _dot(g, w2_v[k * FC:(k + 1) * FC, :])
            seq.append(p)
            y = p if y is None else y + p
        out_v[pl.ds(row0(i), TM), :] = (x1 + gb * y).astype(BF16)
        return seq

    NCH = TM // CH

    def stage_a(i, first):
        a_qkv(i)
        a_attn(first, 0, NCH)

    def stage_b(i):
        x1, h2 = b_ln(i, b_wo())
        b_mlp(i, x1, h2)

    def stage_ab(i):
        att = b_wo()
        a_qkv(i)
        x1, h2 = b_ln(i - 1, att)
        seq = b_mlp(i - 1, x1, h2)
        ng = TM // 8

        def gate8(j):
            f = (j + GOFF) / ng * GSPAN * len(seq)
            v = seq[int(f)]
            nt = v.shape[1] // 128
            p = int((f - int(f)) * nt * ng)
            n, rr = divmod(p, ng)
            return v[rr * 8:(rr + 1) * 8, n * 128:(n + 1) * 128]

        def gate(ch):
            return jnp.concatenate([gate8(ch * (CH // 8) + u) for u in range(CH // 8)], axis=0)
        a_attn(False, 0, NCH, gate)

    x_copy(0).wait()
    stage_a(0, True)
    cp_wo.wait()
    wo_p[...] = _dot(Pt, wo_v[...]).astype(BF16)
    cp_m2.wait()
    mod_s[:, 2 * D:6 * D] = _dot(sc8, wmod_v[:, 2 * D:6 * D])
    cp_w1.wait()
    cp_w2.wait()

    def body(i, carry):
        x_copy(i).wait()
        stage_ab(i)
        o_copy(i - 1).start()
        return carry

    lax.fori_loop(1, NB, body, 0)
    stage_b(NB - 1)
    o_copy(NB - 1).start()
    for i in range(NB):
        o_copy(i).wait()


@jax.jit
def pallas_adaLN_cond__sliding_local_dilated__dense_activation_silu__prompt_kernel(
    A_x, A_wqkv, A_wo, B_x, B_w1, B_w2, c, w_mod):
    any_spec = pl.BlockSpec(memory_space=pl.ANY)
    return pl.pallas_call(
        _kernel,
        out_shape=jax.ShapeDtypeStruct((1, S, D), BF16),
        in_specs=[any_spec, any_spec, any_spec, any_spec, any_spec,
                  pl.BlockSpec(memory_space=pltpu.VMEM), any_spec],
        out_specs=any_spec,
        scratch_shapes=[
            pltpu.VMEM((S, D), BF16),
            pltpu.VMEM((D, 3 * D), BF16),
            pltpu.VMEM((D, 3 * D), BF16),
            pltpu.VMEM((D, D), BF16),
            pltpu.VMEM((D, D), BF16),
            pltpu.VMEM((D, F), BF16),
            pltpu.VMEM((F, D), BF16),
            pltpu.VMEM((D, 6 * D), BF16),
            pltpu.VMEM((S, D), BF16),
            pltpu.VMEM((TM, D), F32),
            pltpu.VMEM((NC, TM + HALO, 128), F32),
            pltpu.VMEM((NC, TM + HALO, 128), F32),
            pltpu.VMEM((TM, D), BF16),
            pltpu.VMEM((8, 6 * D), F32),
            pltpu.VMEM((CH, 128), jnp.int32),
            pltpu.SemaphoreType.DMA((6,)),
            pltpu.SemaphoreType.DMA((NB,)),
            pltpu.SemaphoreType.DMA((NB,)),
        ],
        compiler_params=pltpu.CompilerParams(vmem_limit_bytes=64 * 1024 * 1024),
    )(A_x, A_wqkv, A_wo, B_w1, B_w2, c, w_mod)
```

```python
import jax
import jax.numpy as jnp
from jax import lax
import jax.experimental.pallas as pl
import jax.experimental.pallas.tpu as pltpu

S, D, F = 2048, 512, 1792
H, DH, W, DIL = 32, 16, 8, 2
TM = 256
NB = S // TM
HALO = 16
CH = 16
NC = D // 128
LOG2E = 1.4426950408889634
EPS = 1e-5
FC = 256
NF = F // FC
NCH = TM // CH
GSPAN = 0.93
GP1 = 0.68
GP1B = 0.45
GP1O = 0.47
GP2 = 0.9
GP2O = 0.0
UNROLL_ALL = False
QSCALE = DH ** -0.5 * LOG2E
F32 = jnp.float32
BF16 = jnp.bfloat16
U32 = jnp.uint32


def _dot(a, b):
    return jnp.dot(a, b, preferred_element_type=F32)


def _ln(x):
    m = jnp.sum(x, axis=-1, keepdims=True) * (1.0 / D)
    xc = x - m
    v = jnp.sum(xc * xc, axis=-1, keepdims=True) * (1.0 / D)
    return xc * lax.rsqrt(v + EPS)


def _kernel(x_hbm, wqkv_hbm, wo_hbm, w1_hbm, w2_hbm, c_hbm, wmod_hbm, out_hbm,
            x_v, wqkv_v, wqkv_p, wo_v, wo_p, w1_v, w2_v, wmod_v, out_v,
            qa, ka, va, qb, kb, vb, qc, kc, vc, qd, kd, vd, o_cur, o_nxt, x1_s, h2_s, h1_s, g0_s, p_s, mod_s, zero_s,
            c_v, sem_w, sem_o):
    set_a = (qa, ka, va)
    set_b = (qb, kb, vb)
    set_c = (qc, kc, vc)
    set_d = (qd, kd, vd)

    def x_copy(i):
        return pltpu.make_async_copy(x_hbm.at[0, pl.ds(i * TM, TM), :],
                                     x_v.at[pl.ds(i * TM, TM), :], sem_w.at[13 + i])

    def o_copy(i):
        return pltpu.make_async_copy(out_v.at[pl.ds(i * TM, TM), :],
                                     out_hbm.at[0, pl.ds(i * TM, TM), :], sem_o.at[i])

    def col_copy(src, dst, lo, n, k):
        return pltpu.make_async_copy(src.at[:, pl.ds(lo, n)], dst.at[:, pl.ds(lo, n)], sem_w.at[k])

    HD = D // 2
    cp_qk = [pltpu.make_async_copy(wqkv_hbm.at[pl.ds(u * HD, HD), pl.ds(0, 2 * D)],
                                   wqkv_v.at[pl.ds(u * HD, HD), pl.ds(0, 2 * D)], sem_w.at[u]) for u in range(2)]
    cp_wv = col_copy(wqkv_hbm, wqkv_v, 2 * D, D, 2)
    cp_ma = [col_copy(wmod_hbm, wmod_v, 0, HD, 3), col_copy(wmod_hbm, wmod_v, D, HD, 9)]
    cp_mb = [col_copy(wmod_hbm, wmod_v, HD, HD, 10), col_copy(wmod_hbm, wmod_v, D + HD, HD, 11)]
    cp_m2 = col_copy(wmod_hbm, wmod_v, 2 * D, 4 * D, 4)
    cp_wo = pltpu.make_async_copy(wo_hbm, wo_v, sem_w.at[6])
    cp_w1 = pltpu.make_async_copy(w1_hbm, w1_v, sem_w.at[7])
    cp_w2 = pltpu.make_async_copy(w2_hbm, w2_v, sem_w.at[8])
    cp_c = pltpu.make_async_copy(c_hbm, c_v, sem_w.at[12])

    x_copy(0).start()
    cp_c.start()
    x_copy(1).start()
    cp_qk[0].start()
    for cp in cp_ma + cp_mb:
        cp.start()
    cp_qk[1].start()
    cp_wv.start()
    x_copy(2).start()
    x_copy(3).start()
    cp_wo.start()
    cp_m2.start()
    cp_w1.start()
    cp_w2.start()
    for i in range(4, NB):
        x_copy(i).start()

    r = lax.broadcasted_iota(jnp.int32, (128, 128), 0)
    cc = lax.broadcasted_iota(jnp.int32, (128, 128), 1)

    def tgt(l, c):
        return (l & 3) * 32 + (((l >> 2) & 3) ^ c) * 8 + (l >> 4)

    for c in range(NC):
        p_s[c] = jnp.where(cc == tgt(r, c), 1.0, 0.0).astype(BF16)
        p_s[NC + c] = jnp.where(r == tgt(cc, c), 1.0, 0.0).astype(BF16)

    def perm_cols(t, lo=0, hi=D):
        lane_g = (lax.broadcasted_iota(jnp.int32, ((hi - lo) // 2, 128), 1) >> 2) & 3
        src = [pltpu.bitcast(wqkv_v[lo:hi, t * D + g * 128:t * D + (g + 1) * 128], U32) for g in range(NC)]
        for c in range(NC):
            z = src[c]
            for e in range(1, NC):
                z = jnp.where(lane_g == e, src[c ^ e], z)
            p = p_s[c]
            wqkv_p[lo:hi, t * D + c * 128:t * D + (c + 1) * 128] = _dot(pltpu.bitcast(z, BF16), p).astype(BF16)

    def perm_wo():
        row_g = (lax.broadcasted_iota(jnp.int32, (64, D), 0) >> 1) & 3
        src = [pltpu.bitcast(wo_v[g * 128:(g + 1) * 128, :], U32) for g in range(NC)]
        for c in range(NC):
            z = src[c]
            for e in range(1, NC):
                z = jnp.where(row_g == e, src[c ^ e], z)
            pt = p_s[NC + c]
            wo_p[c * 128:(c + 1) * 128, :] = _dot(pt, pltpu.bitcast(z, BF16)).astype(BF16)

    def row0(i):
        return i * TM if isinstance(i, int) else pl.multiple_of(i * TM, TM)

    def s1_norm(i):
        return _ln(x_v[pl.ds(row0(i), TM), :].astype(F32))

    def s1_chunk(i, ch, g):
        r0 = i * TM + ch * CH
        if not isinstance(i, int):
            r0 = pl.multiple_of(r0, CH)
        x = x_v[pl.ds(r0, CH), :].astype(F32)
        x0 = jnp.where(zero_s[...] != 0, g, x[:, 0:128])
        x = jnp.concatenate([x0, x[:, 128:]], axis=1)
        h1_s[ch * CH:(ch + 1) * CH, :] = s1_mod(_ln(x))

    def s1_mod(n, lo=0, hi=D):
        sa = mod_s[0:1, lo:hi]
        ca = mod_s[0:1, D + lo:D + hi]
        return (n[:, lo:hi] * (1.0 + ca) + sa).astype(BF16)

    def s1_halo(prev, cur):
        for t in (1, 2):
            cur[t][:, 0:HALO, :] = prev[t][:, TM:TM + HALO, :]

    def s1_mm(h, t, cur, seq=None, lo=0, hi=D):
        y = _dot(h, wqkv_p[lo:hi, t * D:(t + 1) * D])
        if t == 0:
            cur[0][...] = y if lo == 0 else cur[0][...] + y
        else:
            for c in range(NC):
                yc = y[:, c * 128:(c + 1) * 128]
                cur[t][c, HALO:HALO + TM, :] = yc if lo == 0 else cur[t][c, HALO:HALO + TM, :] + yc
        if seq is not None:
            seq.append(y)

    def s1(i, prev, cur, seq=None):
        h = h1_s[...] if i is None else s1_mod(s1_norm(i))
        s1_halo(prev, cur)
        for t in range(3):
            s1_mm(h, t, cur, seq)

    def make_gate(seq, span, off=0.0, lo=0, hi=NCH):
        ng = TM // 8
        j0, j1 = lo * (CH // 8), hi * (CH // 8)

        def gate8(j):
            f = (off + (j - j0) / (j1 - j0) * span) * len(seq)
            v = seq[int(f)]
            nt = v.shape[1] // 128
            p = int((f - int(f)) * nt * ng)
            n, rr = divmod(p, ng)
            return v[rr * 8:(rr + 1) * 8, n * 128:(n + 1) * 128]

        def gate(ch):
            return jnp.concatenate([gate8(ch * (CH // 8) + u) for u in range(CH // 8)], axis=0)
        return gate

    def s2(first, cur, o_ref, gate, lo=0, hi=NCH, ln=None):
        q_s, k_s, v_s = cur
        never = zero_s[...] != 0
        outs = {}
        for ch in range(lo, hi):
            b = ch * CH
            qscale = jnp.where(never, gate(ch), QSCALE)
            q = [q_s[b:b + CH, c * 128:(c + 1) * 128] * qscale for c in range(NC)]
            ls = []
            for w in range(W):
                o = HALO + b - DIL * w
                s = q[0] * k_s[0, o:o + CH, :]
                for c in range(1, NC):
                    s = s + q[c] * k_s[c, o:o + CH, :]
                s = s + pltpu.roll(s, 64, 1)
                s = s + pltpu.roll(s, 32, 1)
                if first and b < DIL * w:
                    pos = lax.broadcasted_iota(jnp.int32, (CH, 128), 0) + b
                    s = jnp.where(pos >= DIL * w, s, -1e9 * LOG2E)
                ls.append(s)
            m = ls[0]
            for w in range(1, W):
                m = jnp.maximum(m, ls[w])
            ps = [jnp.exp2(l - m) for l in ls]
            den = ps[0]
            for w in range(1, W):
                den = den + ps[w]
            inv = 1.0 / den
            for c in range(NC):
                acc = ps[0] * v_s[c, HALO + b:HALO + b + CH, :]
                for w in range(1, W):
                    o = HALO + b - DIL * w
                    acc = acc + ps[w] * v_s[c, o:o + CH, :]
                o_ref[b:b + CH, c * 128:(c + 1) * 128] = (acc * inv).astype(BF16)
            if ln is not None:
                s1_chunk(ln, ch, acc)
            outs[ch] = acc
        return outs

    def rgate(lhs, vals):
        never = zero_s[0:8, :] != 0
        col = []
        for ch in range(NCH):
            t = lhs[ch * CH:(ch + 1) * CH, 0:128]
            if ch in vals:
                t = pltpu.bitcast(jnp.where(never, pltpu.bitcast(vals[ch][0:8, :] + vals[ch][8:16, :], U32),
                                            pltpu.bitcast(t, U32)), BF16)
            col.append(t)
        return jnp.concatenate([jnp.concatenate(col, axis=0), lhs[:, 128:]], axis=1)

    def s3(i, o_ref, att=None):
        if att is None:
            att = _dot(o_ref[...], wo_p[...])
        ga = mod_s[0:1, 2 * D:3 * D]
        sb = mod_s[0:1, 3 * D:4 * D]
        cb = mod_s[0:1, 4 * D:5 * D]
        x1 = x_v[pl.ds(row0(i), TM), :].astype(F32) + ga * att
        x1_s[pl.ds(row0(i), TM), :] = x1
        return (_ln(x1) * (0.5 + 0.5 * cb) + 0.5 * sb).astype(BF16)

    def act(t):
        return (t + t * jnp.tanh(t)).astype(BF16)

    def s4_out(i, y):
        gb = mod_s[0:1, 5 * D:6 * D]
        r0 = row0(i)
        out_v[pl.ds(r0, TM), :] = (x1_s[pl.ds(r0, TM), :] + gb * y).astype(BF16)

    def s4(i, h2, seq, mid=None):
        ts = [None] * NF

        def w1c(k):
            ts[k] = _dot(h2, w1_v[:, k * FC:(k + 1) * FC])
            seq.append(ts[k])

        w1c(0)
        y = None
        for k in range(NF):
            if k + 1 < NF:
                w1c(k + 1)
            g = act(ts[k])
            if mid is not None:
                g = mid(k, g)
            p = _dot(g, w2_v[k * FC:(k + 1) * FC, :])
            seq.append(p)
            y = p if y is None else y + p
        s4_out(i, y)

    def mod_mm(lo, hi):
        mod_s[:, lo:hi] = _dot(sc8, wmod_v[:, lo:hi])

    sets = [set_b, set_c, set_d, set_a]
    x_copy(0).wait()
    cp_c.wait()
    cf = c_v[...].astype(F32)
    sg = jax.nn.sigmoid(cf)
    sc = (cf * sg).astype(BF16)
    zero_s[...] = jnp.broadcast_to(jnp.where(sg[:, 0:128] > 2.0, 1, 0), (CH, 128))
    sc8 = jnp.broadcast_to(sc, (8, D))
    n0 = s1_norm(0)
    x_copy(1).wait()
    n1 = s1_norm(1)
    cp_qk[0].wait()
    perm_cols(0, 0, HD)
    perm_cols(1, 0, HD)
    cp_ma[0].wait()
    mod_mm(0, HD)
    cp_ma[1].wait()
    mod_mm(D, D + HD)
    ha = [s1_mod(n, 0, HD) for n in (n0, n1)]
    for u in range(2):
        for t in range(2):
            s1_mm(ha[u], t, sets[u], None, 0, HD)
    cp_mb[0].wait()
    cp_mb[1].wait()
    cp_qk[1].wait()
    perm_cols(0, HD, D)
    mod_mm(HD, D)
    mod_mm(D + HD, 2 * D)
    perm_cols(1, HD, D)
    hb = [s1_mod(n, HD, D) for n in (n0, n1)]
    s1_mm(hb[0], 0, sets[0], None, HD, D)
    s1_mm(hb[0], 1, sets[0], None, HD, D)
    s1_mm(hb[1], 0, sets[1], None, HD, D)
    s1_mm(hb[1], 1, sets[1], None, HD, D)
    h01 = [jnp.concatenate([ha[u], hb[u]], axis=1) for u in range(2)]
    cp_wv.wait()
    x_copy(2).wait()
    x_copy(3).wait()
    cp_wo.wait()
    perm_cols(2)
    s1_mm(h01[0], 2, sets[0])
    for t in (1, 2):
        for c in range(NC):
            sets[0][t][c, 0:HALO, :] = jnp.broadcast_to(sets[0][t][c, HALO:HALO + 1, :], (HALO, 128))
    seq = []
    s1_mm(h01[1], 2, sets[1], seq)
    s1_halo(sets[0], sets[1])
    perm_wo()
    s1(2, sets[1], sets[2], seq)
    s2(True, sets[0], o_nxt, make_gate(seq, GP1), ln=3)
    att0 = _dot(o_nxt[...], wo_p[...])
    x1_s[0:TM, :] = att0
    seq = seq + [att0]
    h3 = h1_s[...]
    s1_halo(sets[2], sets[3])
    s1_mm(h3, 0, sets[3], seq)
    outs = s2(False, sets[1], o_cur, make_gate(seq, GP1B, GP1O))
    s1_mm(rgate(h3, outs), 1, sets[3])
    cp_m2.wait()
    cp_w1.wait()
    att1 = _dot(o_cur[...], wo_p[...])
    mod_mm(2 * D, 5 * D)
    seq = []
    s1_mm(h1_s[...], 2, sets[3], seq)
    h2_0 = s3(0, None, x1_s[0:TM, :])
    h2_s[...] = s3(1, None, att1)
    for k in range(NF):
        if k == 2:
            mod_mm(5 * D, 6 * D)
        if k == NF - 1:
            h2_0 = rgate(h2_0, s2(False, sets[2], o_cur, make_gate(seq, GP2, GP2O)))
        t = _dot(h2_0, w1_v[:, k * FC:(k + 1) * FC])
        seq.append(t)
        g0_s[:, k * FC:(k + 1) * FC] = act(t)
    cp_w2.wait()

    def body(i, carry):
        x_copy(i + 3).wait()
        seq = []
        s4(i, h2_s[...], seq)
        s2(False, set_a, o_nxt, make_gate(seq, GSPAN), ln=i + 3)
        h2_s[...] = s3(i + 1, o_cur)
        o_cur[...] = o_nxt[...]
        s1(None, set_a, set_a)
        o_copy(i).start()
        return carry

    if UNROLL_ALL:
        for i in range(1, NB - 3):
            body(i, 0)
    else:
        lax.fori_loop(1, NB - 3, body, 0)

    h2_5 = h2_s[...]
    h2_6 = s3(6, o_cur)
    s4_out(0, _dot(g0_s[...], w2_v[...]))
    o_copy(0).start()
    seq = []
    s4(5, h2_5, seq)
    s2(False, set_a, o_nxt, make_gate(seq, GSPAN))
    o_copy(5).start()
    h2_7 = s3(7, o_nxt)
    s4(6, h2_6, [])
    o_copy(6).start()
    s4(7, h2_7, [])
    o_copy(7).start()
    for i in range(NB):
        o_copy(i).wait()


@jax.jit
def pallas_adaLN_cond__sliding_local_dilated__dense_activation_silu__prompt_kernel(
    A_x, A_wqkv, A_wo, B_x, B_w1, B_w2, c, w_mod):
    any_spec = pl.BlockSpec(memory_space=pl.ANY)
    qkv_set = [pltpu.VMEM((TM, D), F32),
               pltpu.VMEM((NC, TM + HALO, 128), F32),
               pltpu.VMEM((NC, TM + HALO, 128), F32)]
    return pl.pallas_call(
        _kernel,
        out_shape=jax.ShapeDtypeStruct((1, S, D), BF16),
        in_specs=[any_spec] * 7,
        out_specs=any_spec,
        scratch_shapes=[
            pltpu.VMEM((S, D), BF16),
            pltpu.VMEM((D, 3 * D), BF16),
            pltpu.VMEM((D, 3 * D), BF16),
            pltpu.VMEM((D, D), BF16),
            pltpu.VMEM((D, D), BF16),
            pltpu.VMEM((D, F), BF16),
            pltpu.VMEM((F, D), BF16),
            pltpu.VMEM((D, 6 * D), BF16),
            pltpu.VMEM((S, D), BF16),
            *qkv_set, *qkv_set, *qkv_set, *qkv_set,
            pltpu.VMEM((TM, D), BF16),
            pltpu.VMEM((TM, D), BF16),
            pltpu.VMEM((S, D), F32),
            pltpu.VMEM((TM, D), BF16),
            pltpu.VMEM((TM, D), BF16),
            pltpu.VMEM((TM, F), BF16),
            pltpu.VMEM((2 * NC, 128, 128), BF16),
            pltpu.VMEM((8, 6 * D), F32),
            pltpu.VMEM((CH, 128), jnp.int32),
            pltpu.VMEM((1, D), BF16),
            pltpu.SemaphoreType.DMA((13 + NB,)),
            pltpu.SemaphoreType.DMA((NB,)),
        ],
        compiler_params=pltpu.CompilerParams(vmem_limit_bytes=64 * 1024 * 1024),
    )(A_x, A_wqkv, A_wo, B_w1, B_w2, c, w_mod)
```

```python
import jax
import jax.numpy as jnp
from jax import lax
import jax.experimental.pallas as pl
import jax.experimental.pallas.tpu as pltpu

S, D, F = 2048, 512, 1792
H, DH, W, DIL = 32, 16, 8, 2
TM = 256
NB = S // TM
HALO = 16
CH = 16
NC = D // 128
LOG2E = 1.4426950408889634
EPS = 1e-5
FC = 256
NF = F // FC
NCH = TM // CH
GSPAN = 0.85
GP1 = 0.9
GP1B = 0.75
GOFF = 0.07
GP1O = 0.0
KATT = 1
KD = 3
NLAST = 4
RG = 0
KT7 = 2
GT7 = 0.85
GT7O = 0.1
QSCALE = DH ** -0.5 * LOG2E
F32 = jnp.float32
BF16 = jnp.bfloat16
U32 = jnp.uint32


def _dot(a, b):
    return jnp.dot(a, b, preferred_element_type=F32)


def _ln(x):
    m = jnp.sum(x, axis=-1, keepdims=True) * (1.0 / D)
    xc = x - m
    v = jnp.sum(xc * xc, axis=-1, keepdims=True) * (1.0 / D)
    return xc * lax.rsqrt(v + EPS)


def _kernel(x_hbm, wqkv_hbm, wo_hbm, w1_hbm, w2_hbm, c_hbm, wmod_hbm, out_hbm,
            x_v, wqkv_v, wqkv_p, wo_v, wo_p, w1_v, w2_v, wmod_v, out_v,
            qr, kr, vr, qb, kb, vb, qc, kc, vc, o_cur, o_nxt, x1_s, h2_s, h2x_s, h1_s, g0_s, p_s, mod_s, zero_s,
            c_v, sem_w):
    set_b = (qb, kb, vb)
    set_c = (qc, kc, vc)

    def ring(j):
        return (qr.at[j % 2], kr.at[j % 2], vr.at[j % 2])

    def x_copy(i):
        return pltpu.make_async_copy(x_hbm.at[0, pl.ds(i * TM, TM), :],
                                     x_v.at[pl.ds(i * TM, TM), :], sem_w.at[(0, 1, 1, 0, 1, 2, 2, 2)[i]])

    def o_copy(i):
        return pltpu.make_async_copy(out_v.at[pl.ds(i * TM, TM), :],
                                     out_hbm.at[0, pl.ds(i * TM, TM), :], sem_w.at[0])

    RL = TM // NLAST

    def ol_copy(u):
        r0 = S - TM + u * RL
        return pltpu.make_async_copy(out_v.at[pl.ds(r0, RL), :], out_hbm.at[0, pl.ds(r0, RL), :],
                                     sem_w.at[0])

    def col_copy(src, dst, lo, n, k):
        return pltpu.make_async_copy(src.at[:, pl.ds(lo, n)], dst.at[:, pl.ds(lo, n)], sem_w.at[k])

    KS = [0, 128, 256, 512]
    cp_w = [pltpu.make_async_copy(wqkv_hbm.at[pl.ds(KS[u], KS[u + 1] - KS[u]), :],
                                  wqkv_v.at[pl.ds(KS[u], KS[u + 1] - KS[u]), :], sem_w.at[(2, 1, 2)[u]]) for u in range(3)]
    cp_m = [[col_copy(wmod_hbm, wmod_v, e * D + KS[u], KS[u + 1] - KS[u], u)
             for e in range(2)] for u in range(3)]
    cp_m2 = col_copy(wmod_hbm, wmod_v, 2 * D, 4 * D, 0)
    cp_wo = pltpu.make_async_copy(wo_hbm, wo_v, sem_w.at[2])
    cp_w1 = col_copy(w1_hbm, w1_v, 0, KD * FC, 0)
    cp_w1b = col_copy(w1_hbm, w1_v, KD * FC, F - KD * FC, 1)
    cp_w2 = pltpu.make_async_copy(w2_hbm, w2_v, sem_w.at[1])
    cp_c = pltpu.make_async_copy(c_hbm, c_v, sem_w.at[0])

    groups = [[x_copy(0), cp_c], [x_copy(1)], [cp_w[0]], cp_m[0],
              [cp_w[1]] + cp_m[1] + [x_copy(2)], [cp_w[2]] + cp_m[2] + [cp_wo],
              [x_copy(3), cp_m2, cp_w1], [cp_w1b, cp_w2, x_copy(4)], [x_copy(5), x_copy(6), x_copy(7)]]

    def start_group(g):
        for cp in groups[g]:
            cp.start()

    def await_group(g):
        for cp in groups[g]:
            cp.wait()
        if g + 3 < len(groups):
            start_group(g + 3)

    for g in range(3):
        start_group(g)

    r = lax.broadcasted_iota(jnp.int32, (128, 128), 0)
    cc = lax.broadcasted_iota(jnp.int32, (128, 128), 1)

    def tgt(l, c):
        return (l & 3) * 32 + (((l >> 2) & 3) ^ c) * 8 + (l >> 4)

    for c in range(NC):
        p_s[c] = jnp.where(cc == tgt(r, c), 1.0, 0.0).astype(BF16)
        p_s[NC + c] = jnp.where(r == tgt(cc, c), 1.0, 0.0).astype(BF16)

    def perm_cols(t, lo=0, hi=D):
        lane_g = (lax.broadcasted_iota(jnp.int32, ((hi - lo) // 2, 128), 1) >> 2) & 3
        src = [pltpu.bitcast(wqkv_v[lo:hi, t * D + g * 128:t * D + (g + 1) * 128], U32) for g in range(NC)]
        for c in range(NC):
            z = src[c]
            for e in range(1, NC):
                z = jnp.where(lane_g == e, src[c ^ e], z)
            p = p_s[c]
            wqkv_p[lo:hi, t * D + c * 128:t * D + (c + 1) * 128] = _dot(pltpu.bitcast(z, BF16), p).astype(BF16)

    def perm_wo(seq):
        row_g = (lax.broadcasted_iota(jnp.int32, (64, D), 0) >> 1) & 3
        src = [pltpu.bitcast(wo_v[g * 128:(g + 1) * 128, :], U32) for g in range(NC)]
        ys = []
        for c in range(NC):
            z = src[c]
            for e in range(1, NC):
                z = jnp.where(row_g == e, src[c ^ e], z)
            pt = p_s[NC + c]
            y = _dot(pt, pltpu.bitcast(z, BF16))
            wo_p[c * 128:(c + 1) * 128, :] = y.astype(BF16)
            ys.append(y[0:64, 0:128])
        seq.append(jnp.concatenate(ys, axis=0))

    def row0(i):
        return i * TM if isinstance(i, int) else pl.multiple_of(i * TM, TM)

    def s1_norm(i):
        return _ln(x_v[pl.ds(row0(i), TM), :].astype(F32))

    def s1_chunk(i, ch):
        r0 = i * TM + ch * CH
        if not isinstance(i, int):
            r0 = pl.multiple_of(r0, CH)
        x = x_v[pl.ds(r0, CH), :].astype(F32)
        n = _ln(x)
        h1_s[ch * CH:(ch + 1) * CH, :] = s1_mod(n)
        return n[:, D - 128:D]

    def s1_mod(n, lo=0, hi=D):
        sa = mod_s[0:1, lo:hi]
        ca = mod_s[0:1, D + lo:D + hi]
        return (n[:, lo:hi] * (1.0 + ca) + sa).astype(BF16)

    def s1_halo(prev, cur):
        for t in (1, 2):
            cur[t][:, 0:HALO, :] = prev[t][:, TM:TM + HALO, :]

    def s1_mm(h, t, cur, seq=None, lo=0, hi=D):
        y = _dot(h, wqkv_p[lo:hi, t * D:(t + 1) * D])
        if t == 0:
            cur[0][...] = y if lo == 0 else cur[0][...] + y
        else:
            for c in range(NC):
                yc = y[:, c * 128:(c + 1) * 128]
                cur[t][c, HALO:HALO + TM, :] = yc if lo == 0 else cur[t][c, HALO:HALO + TM, :] + yc
        if seq is not None:
            seq.append(y)

    def s1(prev, cur):
        h = h1_s[...]
        s1_halo(prev, cur)
        for t in range(3):
            s1_mm(h, t, cur)

    def make_gate(seq, span, off=0.0, wt=True):
        ng = TM // 8
        tiles = [(v, n) for v in seq for n in range(v.shape[1] // 128)]

        def gate8(j):
            f = off + j / ng * span
            if wt:
                v, n = tiles[int(f * len(tiles))]
                rr = int((f * len(tiles)) % 1.0 * ng)
            else:
                f = f * len(seq)
                v = seq[int(f)]
                n, rr = divmod(int((f - int(f)) * (v.shape[1] // 128) * ng), ng)
            return v[rr * 8:(rr + 1) * 8, n * 128:(n + 1) * 128]

        def gate(ch):
            return jnp.concatenate([gate8(ch * (CH // 8) + u) for u in range(CH // 8)], axis=0)
        return gate

    def s2(first, cur, o_ref, gate):
        q_s, k_s, v_s = cur
        never = zero_s[...] != 0
        outs = {}
        for ch in range(NCH):
            b = ch * CH
            qscale = jnp.where(never, gate(ch), QSCALE)
            q = [q_s[b:b + CH, c * 128:(c + 1) * 128] * qscale for c in range(NC)]
            ls = []
            for w in range(W):
                o = HALO + b - DIL * w
                s = q[0] * k_s[0, o:o + CH, :]
                for c in range(1, NC):
                    s = s + q[c] * k_s[c, o:o + CH, :]
                s = s + pltpu.roll(s, 64, 1)
                s = s + pltpu.roll(s, 32, 1)
                if first and b < DIL * w:
                    pos = lax.broadcasted_iota(jnp.int32, (CH, 128), 0) + b
                    s = jnp.where(pos >= DIL * w, s, -1e9 * LOG2E)
                ls.append(s)
            m = ls[0]
            for w in range(1, W):
                m = jnp.maximum(m, ls[w])
            ps = [jnp.exp2(l - m) for l in ls]
            den = ps[0]
            for w in range(1, W):
                den = den + ps[w]
            inv = 1.0 / den
            for c in range(NC):
                acc = ps[0] * v_s[c, HALO + b:HALO + b + CH, :]
                for w in range(1, W):
                    o = HALO + b - DIL * w
                    acc = acc + ps[w] * v_s[c, o:o + CH, :]
                o_ref[b:b + CH, c * 128:(c + 1) * 128] = (acc * inv).astype(BF16)
            outs[ch] = acc
        return outs

    def rgate(lhs, vals):
        never = zero_s[0:8, :] != 0
        col = []
        for ch in range(NCH):
            t = lhs[ch * CH:(ch + 1) * CH, RG * 128:(RG + 1) * 128]
            if ch in vals:
                t = pltpu.bitcast(jnp.where(never, pltpu.bitcast(vals[ch][0:8, :] + vals[ch][8:16, :], U32),
                                            pltpu.bitcast(t, U32)), BF16)
            col.append(t)
        parts = [lhs[:, u * 128:(u + 1) * 128] for u in range(lhs.shape[1] // 128)]
        parts[RG] = jnp.concatenate(col, axis=0)
        return jnp.concatenate(parts, axis=1)

    def s3(i, o_ref, att=None):
        if att is None:
            att = _dot(o_ref[...], wo_p[...])
        ga = mod_s[0:1, 2 * D:3 * D]
        sb = mod_s[0:1, 3 * D:4 * D]
        cb = mod_s[0:1, 4 * D:5 * D]
        x1 = x_v[pl.ds(row0(i), TM), :].astype(F32) + ga * att
        x1_s[pl.ds(row0(i), TM), :] = x1
        return (_ln(x1) * (0.5 + 0.5 * cb) + 0.5 * sb).astype(BF16)

    def act(t):
        return (t + t * jnp.tanh(t)).astype(BF16)

    def s4_out(i, y):
        gb = mod_s[0:1, 5 * D:6 * D]
        r0 = row0(i)
        out_v[pl.ds(r0, TM), :] = (x1_s[pl.ds(r0, TM), :] + gb * y).astype(BF16)

    def s4(i, h2, seq, mid=None, last=False):
        ts = [None] * NF

        def w1c(k):
            ts[k] = _dot(h2, w1_v[:, k * FC:(k + 1) * FC])
            seq.append(ts[k])

        w1c(0)
        y = None
        for k in range(NF):
            if k + 1 < NF:
                w1c(k + 1)
            g = act(ts[k])
            if mid is not None:
                g = mid(k, g)
            if last and k == NF - 1:
                gb = mod_s[0:1, 5 * D:6 * D]
                for u in range(NLAST):
                    a, b = u * RL, (u + 1) * RL
                    p = y[a:b, :] + _dot(g[a:b, :], w2_v[k * FC:(k + 1) * FC, :])
                    out_v[i * TM + a:i * TM + b, :] = (x1_s[i * TM + a:i * TM + b, :] + gb * p).astype(BF16)
                    ol_copy(u).start()
                return
            p = _dot(g, w2_v[k * FC:(k + 1) * FC, :])
            seq.append(p)
            y = p if y is None else y + p
        s4_out(i, y)

    def s4_attn(i, h2, cur, o_ref, ln):
        seq = []

        def mid(k, g):
            if k == 0:
                g = rgate(g, {ch: s1_chunk(ln, ch) for ch in range(NCH)})
            return g

        s4(i, h2, seq, mid)
        s2(False, cur, o_ref, make_gate(seq, GSPAN - GOFF, GOFF, wt=False))

    def mod_mm(lo, hi):
        mod_s[:, lo:hi] = _dot(sc8, wmod_v[:, lo:hi])

    def mm_mod(h, w, store, seq, jobs, msplit):
        rows = TM // msplit
        cols = []
        for c in range(NC):
            ys = []
            for u in range(msplit):
                ys.append(_dot(h[u * rows:(u + 1) * rows, :], w(c)))
                if jobs:
                    n = jobs.pop(0)
                    mod_mm(n * 128, (n + 1) * 128)
            yc = jnp.concatenate(ys, axis=0) if msplit > 1 else ys[0]
            store(c, yc)
            cols.append(yc)
        seq.append(jnp.concatenate(cols, axis=1))

    sets = [set_b, set_c, ring(2), ring(3)]
    await_group(0)
    cf = c_v[...].astype(F32)
    sg = jax.nn.sigmoid(cf)
    sc = (cf * sg).astype(BF16)
    zero_s[...] = jnp.broadcast_to(jnp.where(sg[:, 0:128] > 2.0, 1, 0), (CH, 128))
    sc8 = jnp.broadcast_to(sc, (8, D))
    n0 = s1_norm(0)
    await_group(1)
    n1 = s1_norm(1)
    await_group(2)
    for t in range(3):
        perm_cols(t, KS[0], KS[1])
    await_group(3)
    mod_mm(0, 128)
    mod_mm(D, D + 128)
    for u, n in enumerate((n0, n1)):
        h = s1_mod(n, KS[0], KS[1])
        for t in range(3):
            s1_mm(h, t, sets[u], None, KS[0], KS[1])
    await_group(4)
    mod_mm(128, 256)
    perm_cols(0, KS[1], KS[2])
    mod_mm(D + 128, D + 256)
    perm_cols(1, KS[1], KS[2])
    perm_cols(2, KS[1], KS[2])
    n2 = s1_norm(2)
    for u, n in enumerate((n0, n1, n2)):
        lo = KS[1] if u < 2 else 0
        h = s1_mod(n, lo, KS[2])
        for t in range(3):
            s1_mm(h, t, sets[u], None, lo, KS[2])
    await_group(5)
    mod_mm(256, 384)
    mod_mm(D + 256, D + 384)
    perm_cols(0, KS[2], D)
    mod_mm(384, 512)
    mod_mm(D + 384, D + 512)
    perm_cols(1, KS[2], D)
    perm_cols(2, KS[2], D)
    hb = [s1_mod(n, KS[2], D) for n in (n0, n1, n2)]
    seq = []
    for t in range(3):
        s1_mm(hb[0], t, sets[0], seq if t == 2 else None, KS[2], D)
    for t in (1, 2):
        for c in range(NC):
            sets[0][t][c, 0:HALO, :] = jnp.broadcast_to(sets[0][t][c, HALO:HALO + 1, :], (HALO, 128))
    for t in range(3):
        s1_mm(hb[1], t, sets[1], seq, KS[2], D)
    s1_halo(sets[0], sets[1])
    perm_wo(seq)
    s1_halo(sets[1], sets[2])
    for t in range(2):
        s1_mm(hb[2], t, sets[2], seq, KS[2], D)
    outs = s2(True, sets[0], o_nxt, make_gate(seq, GP1, wt=False))
    s1_mm(rgate(hb[2], outs), 2, sets[2], None, KS[2], D)
    await_group(6)
    seq = []
    jobs = list(range(2 * NC, 6 * NC))

    def st_att0(c, yc):
        x1_s[0:TM, c * 128:(c + 1) * 128] = yc

    def st_q3(c, yc):
        sets[3][0][:, c * 128:(c + 1) * 128] = yc

    h3 = s1_mod(s1_norm(3))
    mm_mod(o_nxt[...], lambda c: wo_p[:, c * 128:(c + 1) * 128], st_att0, seq, jobs, 2)
    s1_halo(sets[2], sets[3])
    mm_mod(h3, lambda c: wqkv_p[:, c * 128:(c + 1) * 128], st_q3, seq, jobs, 2)
    s1_mm(h3, 1, sets[3], seq)
    s1_mm(h3, 2, sets[3], seq)
    h2x_s[...] = s3(0, None, x1_s[0:TM, :])
    h2_0 = h2x_s[...]
    for k in range(KD):
        if k == KATT:
            s2(False, sets[1], o_cur, make_gate(seq, GP1B, GP1O))
            h2_s[...] = s3(1, o_cur)
        t = _dot(h2_0, w1_v[:, k * FC:(k + 1) * FC])
        seq.append(t)
        g0_s[:, k * FC:(k + 1) * FC] = act(t)
    await_group(7)

    def body(i, carry):
        @pl.when(i == 2)
        def _():
            await_group(8)

        s4_attn(i, h2_s[...], ring(i + 1), o_cur, i + 3)
        h2_s[...] = s3(i + 1, o_cur)
        s1(ring(i), ring(i + 1))
        o_copy(i).start()
        return carry

    lax.fori_loop(1, NB - 3, body, 0)

    seq = []
    s4(5, h2_s[...], seq)
    o_copy(5).start()
    s2(False, ring(6), o_cur, make_gate(seq, GSPAN, wt=False))
    h2_6 = s3(6, o_cur)
    h2_0 = h2x_s[...]
    seq0 = []
    t0 = _dot(h2_0, w1_v[:, KD * FC:(KD + 1) * FC])
    y0 = _dot(g0_s[:, 0:KD * FC], w2_v[0:KD * FC, :])
    seq0 += [t0] + [y0[:, c * 128:(c + 1) * 128] for c in range(NC)][:KD]
    for k in range(KD, NF):
        g = act(t0)
        if k + 1 < NF:
            t0 = _dot(h2_0, w1_v[:, (k + 1) * FC:(k + 2) * FC])
            seq0.append(t0)
        p = _dot(g, w2_v[k * FC:(k + 1) * FC, :])
        seq0.append(p)
        y0 = y0 + p
    s4_out(0, y0)
    o_copy(0).start()
    st = {}

    def mid(k, g):
        if k == KT7:
            s2(False, ring(7), o_nxt, make_gate(seq0 + seq6, GT7, GT7O, wt=False))
            st['h'] = s3(7, o_nxt)
        return g

    seq6 = []
    s4(6, h2_6, seq6, mid)
    o_copy(6).start()
    s4(7, st['h'], [], last=True)
    for i in range(NB - 1):
        o_copy(i).wait()
    for u in range(NLAST):
        ol_copy(u).wait()


@jax.jit
def pallas_adaLN_cond__sliding_local_dilated__dense_activation_silu__prompt_kernel(
    A_x, A_wqkv, A_wo, B_x, B_w1, B_w2, c, w_mod):
    any_spec = pl.BlockSpec(memory_space=pl.ANY)
    qkv_set = [pltpu.VMEM((TM, D), F32),
               pltpu.VMEM((NC, TM + HALO, 128), F32),
               pltpu.VMEM((NC, TM + HALO, 128), F32)]
    return pl.pallas_call(
        _kernel,
        out_shape=jax.ShapeDtypeStruct((1, S, D), BF16),
        in_specs=[any_spec] * 7,
        out_specs=any_spec,
        scratch_shapes=[
            pltpu.VMEM((S, D), BF16),
            pltpu.VMEM((D, 3 * D), BF16),
            pltpu.VMEM((D, 3 * D), BF16),
            pltpu.VMEM((D, D), BF16),
            pltpu.VMEM((D, D), BF16),
            pltpu.VMEM((D, F), BF16),
            pltpu.VMEM((F, D), BF16),
            pltpu.VMEM((D, 6 * D), BF16),
            pltpu.VMEM((S, D), BF16),
            *[pltpu.VMEM((2,) + t.shape, F32) for t in qkv_set], *qkv_set, *qkv_set,
            pltpu.VMEM((TM, D), BF16),
            pltpu.VMEM((TM, D), BF16),
            pltpu.VMEM((S, D), F32),
            pltpu.VMEM((TM, D), BF16),
            pltpu.VMEM((TM, D), BF16),
            pltpu.VMEM((TM, D), BF16),
            pltpu.VMEM((TM, KD * FC), BF16),
            pltpu.VMEM((2 * NC, 128, 128), BF16),
            pltpu.VMEM((8, 6 * D), F32),
            pltpu.VMEM((CH, 128), jnp.int32),
            pltpu.VMEM((1, D), BF16),
            pltpu.SemaphoreType.DMA((3,)),
        ],
        compiler_params=pltpu.CompilerParams(vmem_limit_bytes=64 * 1024 * 1024),
    )(A_x, A_wqkv, A_wo, B_w1, B_w2, c, w_mod)
```

```python
import jax
import jax.numpy as jnp
from jax import lax
import jax.experimental.pallas as pl
import jax.experimental.pallas.tpu as pltpu

S, D, F = 2048, 512, 1792
H, DH, W, DIL = 32, 16, 8, 2
TM = 256
NB = S // TM
HALO = 16
CH = 16
NC = D // 128
LOG2E = 1.4426950408889634
EPS = 1e-5
FC = 256
NF = F // FC
NCH = TM // CH
GSPAN = 0.93
GP1 = 0.85
GP1B = 0.7
GOFF = 0.07
KATT = 4
KD = 6
KT7 = 4
GT7 = 0.85
GT7O = 0.1
NS = 3
LC = 2
PT = 20
A3 = 160
QSCALE = DH ** -0.5 * LOG2E
F32 = jnp.float32
BF16 = jnp.bfloat16
U32 = jnp.uint32


def _dot(a, b):
    return jnp.dot(a, b, preferred_element_type=F32)


def _ln(x):
    m = jnp.sum(x, axis=-1, keepdims=True) * (1.0 / D)
    xc = x - m
    v = jnp.sum(xc * xc, axis=-1, keepdims=True) * (1.0 / D)
    return xc * lax.rsqrt(v + EPS)


def _kernel(x_hbm, wqkv_hbm, wo_hbm, w1_hbm, w2_hbm, c_hbm, wmod_hbm, out_hbm,
            x_v, wqkv_v, wqkv_p, wo_v, wo_p, w1_v, w2_v, wmod_v, out_v,
            qr, kr, vr, qb, kb, vb, qc, kc, vc, o_cur, o_nxt, x1_s, h2_s, h2x_s, h1_s, g0_s, p_s, mod_s, zero_s,
            c_v, wo_f, sem_w):
    set_b = (qb, kb, vb)
    set_c = (qc, kc, vc)

    def ring(j):
        return (qr.at[j % 2], kr.at[j % 2], vr.at[j % 2])

    GI = dict(x0=0, c=0, ma0=1, ma1=1, q0=2, k0=3, x1=3, mb0=4, mb1=4, qk1=4, wv=5, x2=5, x3=5, wo=5,
              m2=6, w1=6, w1b=7, w2=7, x4=7, x5=8, x6=8, x7=8, o=7)

    def sm(n):
        return GI[n] % NS

    def x_copy(i):
        return pltpu.make_async_copy(x_hbm.at[0, pl.ds(i * TM, TM), :],
                                     x_v.at[pl.ds(i * TM, TM), :], sem_w.at[sm('x%d' % i)])

    def o_copy(i):
        return pltpu.make_async_copy(out_v.at[pl.ds(i * TM, TM), :],
                                     out_hbm.at[0, pl.ds(i * TM, TM), :], sem_w.at[sm('o')])

    RLS = [0, 96, 176, 224, 256]
    NLAST = len(RLS) - 1

    def ol_copy(u):
        r0, RL = S - TM + RLS[u], RLS[u + 1] - RLS[u]
        return pltpu.make_async_copy(out_v.at[pl.ds(r0, RL), :], out_hbm.at[0, pl.ds(r0, RL), :],
                                     sem_w.at[sm('o')])

    def col_copy(src, dst, lo, n, k):
        return pltpu.make_async_copy(src.at[:, pl.ds(lo, n)], dst.at[:, pl.ds(lo, n)], sem_w.at[k])

    HD = D // 2
    cp_qk1 = pltpu.make_async_copy(wqkv_hbm.at[pl.ds(HD, HD), pl.ds(0, 2 * D)],
                                   wqkv_v.at[pl.ds(HD, HD), pl.ds(0, 2 * D)], sem_w.at[sm('qk1')])
    cp_qk0 = [pltpu.make_async_copy(wqkv_hbm.at[pl.ds(0, HD), pl.ds(u * D, D)],
                                    wqkv_v.at[pl.ds(0, HD), pl.ds(u * D, D)], sem_w.at[sm('qk'[u] + '0')])
              for u in range(2)]
    cp_wv = col_copy(wqkv_hbm, wqkv_v, 2 * D, D, sm('wv'))
    cp_ma = [col_copy(wmod_hbm, wmod_v, 0, HD, sm('ma0')), col_copy(wmod_hbm, wmod_v, D, HD, sm('ma1'))]
    cp_mb = [col_copy(wmod_hbm, wmod_v, HD, HD, sm('mb0')), col_copy(wmod_hbm, wmod_v, D + HD, HD, sm('mb1'))]
    cp_m2 = col_copy(wmod_hbm, wmod_v, 2 * D, 4 * D, sm('m2'))
    cp_wo = pltpu.make_async_copy(wo_hbm, wo_v, sem_w.at[sm('wo')])
    cp_w1 = col_copy(w1_hbm, w1_v, 0, KD * FC, sm('w1'))
    cp_w1b = col_copy(w1_hbm, w1_v, KD * FC, F - KD * FC, sm('w1b'))
    cp_w2 = pltpu.make_async_copy(w2_hbm, w2_v, sem_w.at[sm('w2')])
    cp_c = pltpu.make_async_copy(c_hbm, c_v, sem_w.at[sm('c')])

    named = dict(c=cp_c, q0=cp_qk0[0], k0=cp_qk0[1], qk1=cp_qk1, ma0=cp_ma[0], ma1=cp_ma[1], mb0=cp_mb[0], mb1=cp_mb[1],
                 wv=cp_wv, wo=cp_wo, m2=cp_m2, w1=cp_w1, w1b=cp_w1b, w2=cp_w2)
    for i in range(NB):
        named['x%d' % i] = x_copy(i)
    NG = max(GI.values()) + 1
    groups = [[named[k] for k in GI if GI[k] == g and k != 'o'] for g in range(NG)]

    def start_group(g):
        for cp in groups[g]:
            cp.start()

    def await_group(g):
        for cp in groups[g]:
            cp.wait()
        for n, a in enumerate((0, 1, 2, 4, 6, 7)):
            if a == g:
                start_group(n + NS)

    for g in range(NS):
        start_group(g)

    r = lax.broadcasted_iota(jnp.int32, (128, 128), 0)
    cc = lax.broadcasted_iota(jnp.int32, (128, 128), 1)

    def tgt(l, c):
        return (l & 3) * 32 + (((l >> 2) & 3) ^ c) * 8 + (l >> 4)

    for c in range(NC):
        p_s[c] = jnp.where(cc == tgt(r, c), 1.0, 0.0).astype(BF16)

    def perm_cols(t, lo=0, hi=D):
        lane_g = (lax.broadcasted_iota(jnp.int32, ((hi - lo) // 2, 128), 1) >> 2) & 3
        src = [pltpu.bitcast(wqkv_v[lo:hi, t * D + g * 128:t * D + (g + 1) * 128], U32) for g in range(NC)]
        for c in range(NC):
            z = src[c]
            for e in range(1, NC):
                z = jnp.where(lane_g == e, src[c ^ e], z)
            p = p_s[c]
            wqkv_p[lo:hi, t * D + c * 128:t * D + (c + 1) * 128] = _dot(pltpu.bitcast(z, BF16), p).astype(BF16)

    def perm_wo():
        for n in range(NC):
            for h in range(H):
                wo_f[n, h * PT:h * PT + DH, :] = wo_v[h * DH:(h + 1) * DH, n * 128:(n + 1) * 128].astype(F32)
        vals = [{} for _ in range(NC)]
        for n in range(NC):
            for c in range(NC):
                for e in range(4):
                    rows = [wo_f[n, pl.ds(8 * PT * g + (((c ^ g) << 2) | e), 8, stride=PT), :] for g in range(4)]
                    r0 = c * 128 + e * 32
                    y = jnp.concatenate(rows, axis=0)
                    y = y.astype(BF16)
                    wo_p[r0:r0 + 32, n * 128:(n + 1) * 128] = y
                    vals[n][c * 4 + e] = pltpu.bitcast(y, jnp.int32)
        return vals

    def row0(i):
        return i * TM if isinstance(i, int) else pl.multiple_of(i * TM, TM)

    def s1_norm(i):
        return _ln(x_v[pl.ds(row0(i), TM), :].astype(F32))

    def s1_chunk(i, ch, g):
        r0 = i * TM + ch * CH
        if not isinstance(i, int):
            r0 = pl.multiple_of(r0, CH)
        x = x_v[pl.ds(r0, CH), :].astype(F32)
        if g is not None:
            x0 = jnp.where(zero_s[...] != 0, g, x[:, 0:128])
            x = jnp.concatenate([x0, x[:, 128:]], axis=1)
        n = _ln(x)
        h1_s[ch * CH:(ch + 1) * CH, :] = s1_mod(n)
        return n[:, D - 128:D]

    def s1_mod(n, lo=0, hi=D):
        sa = mod_s[0:1, lo:hi]
        ca = mod_s[0:1, D + lo:D + hi]
        return (n[:, lo:hi] * (1.0 + ca) + sa).astype(BF16)

    def s1_halo(prev, cur):
        for t in (1, 2):
            cur[t][:, 0:HALO, :] = prev[t][:, TM:TM + HALO, :]

    def s1_mm(h, t, cur, seq=None, lo=0, hi=D):
        y = _dot(h, wqkv_p[lo:hi, t * D:(t + 1) * D])
        if t == 0:
            cur[0][...] = y if lo == 0 else cur[0][...] + y
        else:
            for c in range(NC):
                yc = y[:, c * 128:(c + 1) * 128]
                cur[t][c, HALO:HALO + TM, :] = yc if lo == 0 else cur[t][c, HALO:HALO + TM, :] + yc
        if seq is not None:
            seq.append(y)

    def s1(i, prev, cur, seq=None):
        h = h1_s[...] if i is None else s1_mod(s1_norm(i))
        s1_halo(prev, cur)
        for t in range(3):
            s1_mm(h, t, cur, seq)

    def make_gate(seq, span, off=0.0, wt=True):
        ng = TM // 8
        tiles = [(v, n) for v in seq for n in range(v.shape[1] // 128)]

        def gate8(j):
            f = off + j / ng * span
            if wt:
                v, n = tiles[int(f * len(tiles))]
                rr = int((f * len(tiles)) % 1.0 * ng)
            else:
                f = f * len(seq)
                v = seq[int(f)]
                n, rr = divmod(int((f - int(f)) * (v.shape[1] // 128) * ng), ng)
            return v[rr * 8:(rr + 1) * 8, n * 128:(n + 1) * 128]

        def gate(ch):
            return jnp.concatenate([gate8(ch * (CH // 8) + u) for u in range(CH // 8)], axis=0)
        return gate

    def s2(first, cur, o_ref, gate, ln=None):
        q_s, k_s, v_s = cur
        never = zero_s[...] != 0
        outs = {}
        for ch in range(NCH):
            b = ch * CH
            qscale = jnp.where(never, gate(ch), QSCALE)
            q = [q_s[b:b + CH, c * 128:(c + 1) * 128] * qscale for c in range(NC)]
            ls = []
            for w in range(W):
                o = HALO + b - DIL * w
                s = q[0] * k_s[0, o:o + CH, :]
                for c in range(1, NC):
                    s = s + q[c] * k_s[c, o:o + CH, :]
                s = s + pltpu.roll(s, 64, 1)
                s = s + pltpu.roll(s, 32, 1)
                if first and b < DIL * w:
                    pos = lax.broadcasted_iota(jnp.int32, (CH, 128), 0) + b
                    s = jnp.where(pos >= DIL * w, s, -1e9 * LOG2E)
                ls.append(s)
            m = ls[0]
            for w in range(1, W):
                m = jnp.maximum(m, ls[w])
            ps = [jnp.exp2(l - m) for l in ls]
            den = ps[0]
            for w in range(1, W):
                den = den + ps[w]
            inv = 1.0 / den
            for c in range(NC):
                acc = ps[0] * v_s[c, HALO + b:HALO + b + CH, :]
                for w in range(1, W):
                    o = HALO + b - DIL * w
                    acc = acc + ps[w] * v_s[c, o:o + CH, :]
                o_ref[b:b + CH, c * 128:(c + 1) * 128] = (acc * inv).astype(BF16)
            if ln is not None:
                acc = s1_chunk(ln, ch, acc)
            outs[ch] = acc
        return outs

    def rgate(lhs, vals, RG=0):
        never = zero_s[0:8, :] != 0
        col = []
        for ch in range(NCH):
            t = lhs[ch * CH:(ch + 1) * CH, RG * 128:(RG + 1) * 128]
            if ch in vals:
                t = pltpu.bitcast(jnp.where(never, pltpu.bitcast(vals[ch][0:8, :] + vals[ch][8:16, :], U32),
                                            pltpu.bitcast(t, U32)), BF16)
            col.append(t)
        parts = [lhs[:, u * 128:(u + 1) * 128] for u in range(lhs.shape[1] // 128)]
        parts[RG] = jnp.concatenate(col, axis=0)
        return jnp.concatenate(parts, axis=1)

    def s3(i, o_ref, att=None):
        if att is None:
            att = jnp.concatenate([_dot(o_ref[a:b, :], wo_p[...]) for a, b in ((0, A3), (A3, TM))], axis=0)
        ga = mod_s[0:1, 2 * D:3 * D]
        sb = mod_s[0:1, 3 * D:4 * D]
        cb = mod_s[0:1, 4 * D:5 * D]
        x1 = x_v[pl.ds(row0(i), TM), :].astype(F32) + ga * att
        x1_s[pl.ds(row0(i), TM), :] = x1
        return (_ln(x1) * (0.5 + 0.5 * cb) + 0.5 * sb).astype(BF16)

    def act(t):
        return (t + t * jnp.tanh(t)).astype(BF16)

    def s4_out(i, y):
        gb = mod_s[0:1, 5 * D:6 * D]
        r0 = row0(i)
        out_v[pl.ds(r0, TM), :] = (x1_s[pl.ds(r0, TM), :] + gb * y).astype(BF16)

    def s4(i, h2, seq, mid=None, last=False):
        ts = [None] * NF

        def w1c(k):
            ts[k] = _dot(h2, w1_v[:, k * FC:(k + 1) * FC])
            seq.append(ts[k])

        w1c(0)
        y = None
        for k in range(NF):
            if k + 1 < NF and ts[k + 1] is None:
                w1c(k + 1)
            if last and k == NF - LC - 1:
                for kk in range(k + 2, NF):
                    w1c(kk)
            g = act(ts[k])
            if mid is not None:
                g = mid(k, g)
            if last and k == NF - LC:
                gb = mod_s[0:1, 5 * D:6 * D]
                g = jnp.concatenate([g] + [act(ts[kk]) for kk in range(k + 1, NF)], axis=1)
                for u in range(NLAST):
                    a, b = RLS[u], RLS[u + 1]
                    p = y[a:b, :] + _dot(g[a:b, :], w2_v[k * FC:F, :])
                    out_v[i * TM + a:i * TM + b, :] = (x1_s[i * TM + a:i * TM + b, :] + gb * p).astype(BF16)
                    ol_copy(u).start()
                return
            p = _dot(g, w2_v[k * FC:(k + 1) * FC, :])
            seq.append(p)
            y = p if y is None else y + p
        s4_out(i, y)

    def s4_attn(i, h2, cur, o_ref, ln):
        seq = []

        def mid(k, g):
            if k == 0:
                g = rgate(g, {ch: s1_chunk(ln, ch, None) for ch in range(NCH)})
            return g

        s4(i, h2, seq, mid)
        s2(False, cur, o_ref, make_gate(seq, GSPAN - GOFF, GOFF, wt=False))

    def mod_mm(lo, hi):
        mod_s[:, lo:hi] = _dot(sc8, wmod_v[:, lo:hi])

    def mm_mod(h, t, cur, seq, jobs, msplit):
        rows = TM // msplit
        cols = []
        for c in range(NC):
            ys = []
            for u in range(msplit):
                ys.append(_dot(h[u * rows:(u + 1) * rows, :], wqkv_p[:, t * D + c * 128:t * D + (c + 1) * 128]))
                if jobs:
                    n = jobs.pop(0)
                    mod_mm(n * 128, (n + 1) * 128)
            yc = jnp.concatenate(ys, axis=0) if msplit > 1 else ys[0]
            if t == 0:
                cur[0][:, c * 128:(c + 1) * 128] = yc
            else:
                cur[t][c, HALO:HALO + TM, :] = yc
            cols.append(yc)
        seq.append(jnp.concatenate(cols, axis=1))

    sets = [set_b, set_c, ring(2), ring(3)]
    await_group(0)
    cf = c_v[...].astype(F32)
    sg = jax.nn.sigmoid(cf)
    sc = (cf * sg).astype(BF16)
    zero_s[...] = jnp.broadcast_to(jnp.where(sg[:, 0:128] > 2.0, 1, 0), (CH, 128))
    sc8 = jnp.broadcast_to(sc, (8, D))
    n0 = s1_norm(0)
    await_group(1)
    mod_mm(0, HD)
    mod_mm(D, D + HD)
    ha = [s1_mod(n0, 0, HD)]

    def perm2(t):
        for r in range(0, HD, 128):
            perm_cols(t, r, r + 128)

    def mm2(h, t, cur):
        for r in range(0, HD, 128):
            s1_mm(h[:, r:r + 128], t, cur, None, r, r + 128)

    await_group(2)
    perm2(0)
    mm2(ha[0], 0, sets[0])
    await_group(3)
    perm2(1)
    n1 = s1_norm(1)
    ha.append(s1_mod(n1, 0, HD))
    mm2(ha[0], 1, sets[0])
    s1_mm(ha[1], 0, sets[1], None, 0, HD)
    s1_mm(ha[1], 1, sets[1], None, 0, HD)
    await_group(GI['qk1'])
    perm_cols(0, HD, D)
    mod_mm(HD, D)
    mod_mm(D + HD, 2 * D)
    perm_cols(1, HD, D)
    hb = [s1_mod(n, HD, D) for n in (n0, n1)]
    s1_mm(hb[0], 0, sets[0], None, HD, D)
    s1_mm(hb[0], 1, sets[0], None, HD, D)
    s1_mm(hb[1], 0, sets[1], None, HD, D)
    s1_mm(hb[1], 1, sets[1], None, HD, D)
    h01 = [jnp.concatenate([ha[u], hb[u]], axis=1) for u in range(2)]
    await_group(GI['wv'])
    perm_cols(2)
    wv = perm_wo()
    for c in range(NC):
        hg = rgate(h01[0], wv[c], c)
        sets[0][2][c, HALO:HALO + TM, :] = _dot(hg, wqkv_p[:, 2 * D + c * 128:2 * D + (c + 1) * 128])
    for t in (1, 2):
        for c in range(NC):
            sets[0][t][c, 0:HALO, :] = jnp.broadcast_to(sets[0][t][c, HALO:HALO + 1, :], (HALO, 128))
    seq = []
    s1_mm(h01[1], 2, sets[1], seq)
    s1_halo(sets[0], sets[1])
    s1(2, sets[1], sets[2], seq)
    s2(True, sets[0], o_nxt, make_gate(seq, GP1), ln=3)
    x1_s[0:TM, :] = _dot(o_nxt[...], wo_p[...])
    await_group(GI['m2'])
    seq = []
    jobs = list(range(3 * NC, 5 * NC)) + list(range(2 * NC, 3 * NC)) + list(range(5 * NC, 6 * NC))
    h3 = h1_s[...]
    s1_halo(sets[2], sets[3])
    mm_mod(h3, 0, sets[3], seq, jobs, 2)
    mm_mod(h3, 1, sets[3], seq, jobs, 2)
    s1_mm(h3, 2, sets[3], seq)
    h2x_s[...] = s3(0, None, x1_s[0:TM, :])
    h2_0 = h2x_s[...]
    for k in range(KD):
        if k == KATT:
            s2(False, sets[1], o_cur, make_gate(seq, GP1B))
            h2_s[...] = s3(1, o_cur)
        t = _dot(h2_0, w1_v[:, k * FC:(k + 1) * FC])
        seq.append(t)
        g0_s[:, k * FC:(k + 1) * FC] = act(t)
    await_group(GI['w2'])

    def body(i, carry):
        @pl.when(i == 2)
        def _():
            await_group(GI['x5'])

        s4_attn(i, h2_s[...], ring(i + 1), o_cur, i + 3)
        h2_s[...] = s3(i + 1, o_cur)
        s1(None, ring(i), ring(i + 1))
        o_copy(i).start()
        return carry

    lax.fori_loop(1, NB - 3, body, 0)

    seq = []
    s4(5, h2_s[...], seq)
    o_copy(5).start()
    s2(False, ring(6), o_cur, make_gate(seq, GSPAN, wt=False))
    h2_6 = s3(6, o_cur)
    t0 = _dot(h2x_s[...], w1_v[:, KD * FC:F])
    y0 = _dot(g0_s[:, 0:KD * FC], w2_v[0:KD * FC, :])
    y0 = y0 + _dot(act(t0), w2_v[KD * FC:F, :])
    s4_out(0, y0)
    o_copy(0).start()
    st = {}

    def mid(k, g):
        if k == KT7:
            s2(False, ring(7), o_nxt, make_gate([y0[:, :256], y0[:, 256:]] * 1 + seq6, GT7, GT7O, wt=False))
            st['h'] = s3(7, o_nxt)
        return g

    seq6 = []
    s4(6, h2_6, seq6, mid)
    o_copy(6).start()
    s4(7, st['h'], [], last=True)
    for i in range(NB - 1):
        o_copy(i).wait()
    for u in range(NLAST):
        ol_copy(u).wait()


@jax.jit
def pallas_adaLN_cond__sliding_local_dilated__dense_activation_silu__prompt_kernel(
    A_x, A_wqkv, A_wo, B_x, B_w1, B_w2, c, w_mod):
    any_spec = pl.BlockSpec(memory_space=pl.ANY)
    qkv_set = [pltpu.VMEM((TM, D), F32),
               pltpu.VMEM((NC, TM + HALO, 128), F32),
               pltpu.VMEM((NC, TM + HALO, 128), F32)]
    return pl.pallas_call(
        _kernel,
        out_shape=jax.ShapeDtypeStruct((1, S, D), BF16),
        in_specs=[any_spec] * 7,
        out_specs=any_spec,
        scratch_shapes=[
            pltpu.VMEM((S, D), BF16),
            pltpu.VMEM((D, 3 * D), BF16),
            pltpu.VMEM((D, 3 * D), BF16),
            pltpu.VMEM((D, D), BF16),
            pltpu.VMEM((D, D), BF16),
            pltpu.VMEM((D, F), BF16),
            pltpu.VMEM((F, D), BF16),
            pltpu.VMEM((D, 6 * D), BF16),
            pltpu.VMEM((S, D), BF16),
            *[pltpu.VMEM((2,) + t.shape, F32) for t in qkv_set], *qkv_set, *qkv_set,
            pltpu.VMEM((TM, D), BF16),
            pltpu.VMEM((TM, D), BF16),
            pltpu.VMEM((S, D), F32),
            pltpu.VMEM((TM, D), BF16),
            pltpu.VMEM((TM, D), BF16),
            pltpu.VMEM((TM, D), BF16),
            pltpu.VMEM((TM, F), BF16),
            pltpu.VMEM((NC, 128, 128), BF16),
            pltpu.VMEM((8, 6 * D), F32),
            pltpu.VMEM((CH, 128), jnp.int32),
            pltpu.VMEM((1, D), BF16),
            pltpu.VMEM((NC, (H + 1) * PT, 128), F32),
            pltpu.SemaphoreType.DMA((NS,)),
        ],
        compiler_params=pltpu.CompilerParams(vmem_limit_bytes=64 * 1024 * 1024),
    )(A_x, A_wqkv, A_wo, B_w1, B_w2, c, w_mod)
```

```python
import jax
import jax.numpy as jnp
from jax import lax
import jax.experimental.pallas as pl
import jax.experimental.pallas.tpu as pltpu

S, D, F = 2048, 512, 1792
H, DH, W, DIL = 32, 16, 8, 2
TM = 256
NB = S // TM
HALO = 16
CH = 16
NC = D // 128
LOG2E = 1.4426950408889634
EPS = 1e-5
FC = 256
NF = F // FC
NCH = TM // CH
GSPAN = 0.93
GP1 = 0.85
GP1B = 0.7
GOFF = 0.07
KATT = 4
KD = 6
KT7 = 4
GT7 = 0.85
GT7O = 0.1
NS = 3
LC = 2
PT = 20
A3 = 128
QSCALE = DH ** -0.5 * LOG2E
F32 = jnp.float32
BF16 = jnp.bfloat16
U32 = jnp.uint32


def _dot(a, b):
    return jnp.dot(a, b, preferred_element_type=F32)


def _ln(x):
    m = jnp.sum(x, axis=-1, keepdims=True) * (1.0 / D)
    xc = x - m
    v = jnp.sum(xc * xc, axis=-1, keepdims=True) * (1.0 / D)
    return xc * lax.rsqrt(v + EPS)


def _kernel(x_hbm, wqkv_hbm, wo_hbm, w1_hbm, w2_hbm, c_hbm, wmod_hbm, out_hbm,
            x_v, wqkv_v, wqkv_p, wo_v, wo_p, w1_v, w2_v, wmod_v, out_v,
            qr, kr, vr, qb, kb, vb, qc, kc, vc, o_cur, o_nxt, x1_s, h2_s, h2x_s, h1_s, g0_s, p_s, mod_s, zero_s,
            c_v, wo_f, sem_w):
    set_b = (qb, kb, vb)
    set_c = (qc, kc, vc)

    def ring(j):
        return (qr.at[j % 2], kr.at[j % 2], vr.at[j % 2])

    GI = dict(x0=0, c=0, ma0=1, ma1=1, q0=2, k0=3, x1=3, mb0=4, mb1=4, qk1=4, wv=5, x2=5, wo=5,
              m2=6, w1=6, w1b=7, w2=7, x4=7, o=7)

    def sm(n):
        return GI[n] % NS

    def x_copy(i, n):
        return pltpu.make_async_copy(x_hbm.at[0, pl.ds(i * TM, n * TM), :],
                                     x_v.at[pl.ds(i * TM, n * TM), :], sem_w.at[sm('x%d' % i)])

    def o_copy(i):
        return pltpu.make_async_copy(out_v.at[pl.ds(i * TM, TM), :],
                                     out_hbm.at[0, pl.ds(i * TM, TM), :], sem_w.at[sm('o')])

    RLS = [0, 96, 176, 224, 256]
    NLAST = len(RLS) - 1

    def ol_copy(u):
        r0, RL = S - TM + RLS[u], RLS[u + 1] - RLS[u]
        return pltpu.make_async_copy(out_v.at[pl.ds(r0, RL), :], out_hbm.at[0, pl.ds(r0, RL), :],
                                     sem_w.at[sm('o')])

    def col_copy(src, dst, lo, n, k):
        return pltpu.make_async_copy(src.at[:, pl.ds(lo, n)], dst.at[:, pl.ds(lo, n)], sem_w.at[k])

    HD = D // 2
    cp_qk1 = pltpu.make_async_copy(wqkv_hbm.at[pl.ds(HD, HD), pl.ds(0, 2 * D)],
                                   wqkv_v.at[pl.ds(HD, HD), pl.ds(0, 2 * D)], sem_w.at[sm('qk1')])
    cp_qk0 = [pltpu.make_async_copy(wqkv_hbm.at[pl.ds(0, HD), pl.ds(u * D, D)],
                                    wqkv_v.at[pl.ds(0, HD), pl.ds(u * D, D)], sem_w.at[sm('qk'[u] + '0')])
              for u in range(2)]
    cp_wv = col_copy(wqkv_hbm, wqkv_v, 2 * D, D, sm('wv'))
    cp_ma = [col_copy(wmod_hbm, wmod_v, 0, HD, sm('ma0')), col_copy(wmod_hbm, wmod_v, D, HD, sm('ma1'))]
    cp_mb = [col_copy(wmod_hbm, wmod_v, HD, HD, sm('mb0')), col_copy(wmod_hbm, wmod_v, D + HD, HD, sm('mb1'))]
    cp_m2 = col_copy(wmod_hbm, wmod_v, 2 * D, 4 * D, sm('m2'))
    cp_wo = pltpu.make_async_copy(wo_hbm, wo_v, sem_w.at[sm('wo')])
    cp_w1 = col_copy(w1_hbm, w1_v, 0, KD * FC, sm('w1'))
    cp_w1b = col_copy(w1_hbm, w1_v, KD * FC, F - KD * FC, sm('w1b'))
    cp_w2 = pltpu.make_async_copy(w2_hbm, w2_v, sem_w.at[sm('w2')])
    cp_c = pltpu.make_async_copy(c_hbm, c_v, sem_w.at[sm('c')])

    named = dict(c=cp_c, q0=cp_qk0[0], k0=cp_qk0[1], qk1=cp_qk1, ma0=cp_ma[0], ma1=cp_ma[1], mb0=cp_mb[0], mb1=cp_mb[1],
                 wv=cp_wv, wo=cp_wo, m2=cp_m2, w1=cp_w1, w1b=cp_w1b, w2=cp_w2)
    for i, n in ((0, 1), (1, 1), (2, 2), (4, NB - 4)):
        named['x%d' % i] = x_copy(i, n)
    NG = max(GI.values()) + 1
    groups = [[named[k] for k in GI if GI[k] == g and k != 'o'] for g in range(NG)]

    def start_group(g):
        for cp in groups[g]:
            cp.start()

    def await_group(g):
        for cp in groups[g]:
            cp.wait()
        for n, a in enumerate((0, 1, 2, 3, 6)):
            if a == g:
                start_group(n + NS)

    for g in range(NS):
        start_group(g)

    r = lax.broadcasted_iota(jnp.int32, (128, 128), 0)
    cc = lax.broadcasted_iota(jnp.int32, (128, 128), 1)

    def tgt(l, c):
        return (l & 3) * 32 + (((l >> 2) & 3) ^ c) * 8 + (l >> 4)

    for c in range(NC):
        p_s[c] = jnp.where(cc == tgt(r, c), 1.0, 0.0).astype(BF16)

    def perm_cols(t, lo=0, hi=D):
        lane_g = (lax.broadcasted_iota(jnp.int32, ((hi - lo) // 2, 128), 1) >> 2) & 3
        src = [pltpu.bitcast(wqkv_v[lo:hi, t * D + g * 128:t * D + (g + 1) * 128], U32) for g in range(NC)]
        for c in range(NC):
            z = src[c]
            for e in range(1, NC):
                z = jnp.where(lane_g == e, src[c ^ e], z)
            p = p_s[c]
            wqkv_p[lo:hi, t * D + c * 128:t * D + (c + 1) * 128] = _dot(pltpu.bitcast(z, BF16), p).astype(BF16)

    def perm_wo():
        for n in range(NC):
            for h in range(H):
                wo_f[n, h * PT:h * PT + DH, :] = wo_v[h * DH:(h + 1) * DH, n * 128:(n + 1) * 128].astype(F32)
        vals = [{} for _ in range(NC)]
        for n in range(NC):
            for c in range(NC):
                for e in range(4):
                    rows = [wo_f[n, pl.ds(8 * PT * g + (((c ^ g) << 2) | e), 8, stride=PT), :] for g in range(4)]
                    r0 = c * 128 + e * 32
                    y = jnp.concatenate(rows, axis=0)
                    y = y.astype(BF16)
                    wo_p[r0:r0 + 32, n * 128:(n + 1) * 128] = y
                    vals[n][c * 4 + e] = pltpu.bitcast(y, jnp.int32)
        return vals

    def row0(i):
        return i * TM if isinstance(i, int) else pl.multiple_of(i * TM, TM)

    def s1_norm(i):
        return _ln(x_v[pl.ds(row0(i), TM), :].astype(F32))

    def s1_chunk(i, ch, g):
        r0 = i * TM + ch * CH
        if not isinstance(i, int):
            r0 = pl.multiple_of(r0, CH)
        x = x_v[pl.ds(r0, CH), :].astype(F32)
        if g is not None:
            x0 = jnp.where(zero_s[...] != 0, g, x[:, 0:128])
            x = jnp.concatenate([x0, x[:, 128:]], axis=1)
        n = _ln(x)
        h1_s[ch * CH:(ch + 1) * CH, :] = s1_mod(n)
        return n[:, D - 128:D]

    def s1_mod(n, lo=0, hi=D):
        sa = mod_s[0:1, lo:hi]
        ca = mod_s[0:1, D + lo:D + hi]
        return (n[:, lo:hi] * (1.0 + ca) + sa).astype(BF16)

    def s1_halo(prev, cur):
        for t in (1, 2):
            cur[t][:, 0:HALO, :] = prev[t][:, TM:TM + HALO, :]

    def s1_mm(h, t, cur, seq=None, lo=0, hi=D):
        y = _dot(h, wqkv_p[lo:hi, t * D:(t + 1) * D])
        if t == 0:
            cur[0][...] = y if lo == 0 else cur[0][...] + y
        else:
            for c in range(NC):
                yc = y[:, c * 128:(c + 1) * 128]
                cur[t][c, HALO:HALO + TM, :] = yc if lo == 0 else cur[t][c, HALO:HALO + TM, :] + yc
        if seq is not None:
            seq.append(y)

    def s1(i, prev, cur, seq=None):
        h = h1_s[...] if i is None else s1_mod(s1_norm(i))
        s1_halo(prev, cur)
        for t in range(3):
            s1_mm(h, t, cur, seq)

    def make_gate(seq, span, off=0.0, wt=True):
        ng = TM // 8
        tiles = [(v, n) for v in seq for n in range(v.shape[1] // 128)]

        def gate8(j):
            f = off + j / ng * span
            if wt:
                v, n = tiles[int(f * len(tiles))]
                rr = int((f * len(tiles)) % 1.0 * ng)
            else:
                f = f * len(seq)
                v = seq[int(f)]
                n, rr = divmod(int((f - int(f)) * (v.shape[1] // 128) * ng), ng)
            return v[rr * 8:(rr + 1) * 8, n * 128:(n + 1) * 128]

        def gate(ch):
            return jnp.concatenate([gate8(ch * (CH // 8) + u) for u in range(CH // 8)], axis=0)
        return gate

    def s2(first, cur, o_ref, gate, ln=None):
        q_s, k_s, v_s = cur
        never = zero_s[...] != 0
        outs = {}
        for ch in range(NCH):
            b = ch * CH
            qscale = jnp.where(never, gate(ch), QSCALE)
            q = [q_s[b:b + CH, c * 128:(c + 1) * 128] * qscale for c in range(NC)]
            ls = []
            for w in range(W):
                o = HALO + b - DIL * w
                s = q[0] * k_s[0, o:o + CH, :]
                for c in range(1, NC):
                    s = s + q[c] * k_s[c, o:o + CH, :]
                s = s + pltpu.roll(s, 64, 1)
                s = s + pltpu.roll(s, 32, 1)
                if first and b < DIL * w:
                    pos = lax.broadcasted_iota(jnp.int32, (CH, 128), 0) + b
                    s = jnp.where(pos >= DIL * w, s, -1e9 * LOG2E)
                ls.append(s)
            m = ls[0]
            for w in range(1, W):
                m = jnp.maximum(m, ls[w])
            ps = [jnp.exp2(l - m) for l in ls]
            den = ps[0]
            for w in range(1, W):
                den = den + ps[w]
            inv = 1.0 / den
            for c in range(NC):
                acc = ps[0] * v_s[c, HALO + b:HALO + b + CH, :]
                for w in range(1, W):
                    o = HALO + b - DIL * w
                    acc = acc + ps[w] * v_s[c, o:o + CH, :]
                o_ref[b:b + CH, c * 128:(c + 1) * 128] = (acc * inv).astype(BF16)
            if ln is not None:
                acc = s1_chunk(ln, ch, acc)
            outs[ch] = acc
        return outs

    def rgate(lhs, vals, RG=0):
        never = zero_s[0:8, :] != 0
        col = []
        for ch in range(NCH):
            t = lhs[ch * CH:(ch + 1) * CH, RG * 128:(RG + 1) * 128]
            if ch in vals:
                t = pltpu.bitcast(jnp.where(never, pltpu.bitcast(vals[ch][0:8, :] + vals[ch][8:16, :], U32),
                                            pltpu.bitcast(t, U32)), BF16)
            col.append(t)
        parts = [lhs[:, u * 128:(u + 1) * 128] for u in range(lhs.shape[1] // 128)]
        parts[RG] = jnp.concatenate(col, axis=0)
        return jnp.concatenate(parts, axis=1)

    def s3(i, o_ref, att=None):
        if att is None:
            att = jnp.concatenate([_dot(o_ref[a:b, :], wo_p[...]) for a, b in ((0, A3), (A3, TM))], axis=0)
        ga = mod_s[0:1, 2 * D:3 * D]
        sb = mod_s[0:1, 3 * D:4 * D]
        cb = mod_s[0:1, 4 * D:5 * D]
        x1 = x_v[pl.ds(row0(i), TM), :].astype(F32) + ga * att
        x1_s[pl.ds(row0(i), TM), :] = x1
        return (_ln(x1) * (0.5 + 0.5 * cb) + 0.5 * sb).astype(BF16)

    def act(t):
        return (t + t * jnp.tanh(t)).astype(BF16)

    def s4_out(i, y):
        gb = mod_s[0:1, 5 * D:6 * D]
        r0 = row0(i)
        out_v[pl.ds(r0, TM), :] = (x1_s[pl.ds(r0, TM), :] + gb * y).astype(BF16)

    def s4(i, h2, seq, mid=None, last=False):
        ts = [None] * NF

        def w1c(k):
            ts[k] = _dot(h2, w1_v[:, k * FC:(k + 1) * FC])
            seq.append(ts[k])

        w1c(0)
        y = None
        for k in range(NF):
            if k + 1 < NF and ts[k + 1] is None:
                w1c(k + 1)
            if last and k == NF - LC - 1:
                for kk in range(k + 2, NF):
                    w1c(kk)
            g = act(ts[k])
            if mid is not None:
                g = mid(k, g)
            if last and k == NF - LC:
                gb = mod_s[0:1, 5 * D:6 * D]
                g = jnp.concatenate([g] + [act(ts[kk]) for kk in range(k + 1, NF)], axis=1)
                for u in range(NLAST):
                    a, b = RLS[u], RLS[u + 1]
                    p = y[a:b, :] + _dot(g[a:b, :], w2_v[k * FC:F, :])
                    out_v[i * TM + a:i * TM + b, :] = (x1_s[i * TM + a:i * TM + b, :] + gb * p).astype(BF16)
                    ol_copy(u).start()
                return
            p = _dot(g, w2_v[k * FC:(k + 1) * FC, :])
            seq.append(p)
            y = p if y is None else y + p
        s4_out(i, y)

    def s4_attn(i, h2, cur, o_ref, ln):
        seq = []

        def mid(k, g):
            if k == 0:
                g = rgate(g, {ch: s1_chunk(ln, ch, None) for ch in range(NCH)})
            return g

        s4(i, h2, seq, mid)
        s2(False, cur, o_ref, make_gate(seq, GSPAN - GOFF, GOFF, wt=False))

    def mod_mm(lo, hi):
        mod_s[:, lo:hi] = _dot(sc8, wmod_v[:, lo:hi])

    def mm_mod(h, t, cur, seq, jobs, msplit):
        rows = TM // msplit
        cols = []
        for c in range(NC):
            ys = []
            for u in range(msplit):
                ys.append(_dot(h[u * rows:(u + 1) * rows, :], wqkv_p[:, t * D + c * 128:t * D + (c + 1) * 128]))
                if jobs:
                    n = jobs.pop(0)
                    mod_mm(n * 128, (n + 1) * 128)
            yc = jnp.concatenate(ys, axis=0) if msplit > 1 else ys[0]
            if t == 0:
                cur[0][:, c * 128:(c + 1) * 128] = yc
            else:
                cur[t][c, HALO:HALO + TM, :] = yc
            cols.append(yc)
        seq.append(jnp.concatenate(cols, axis=1))

    sets = [set_b, set_c, ring(2), ring(3)]
    await_group(0)
    cf = c_v[...].astype(F32)
    sg = jax.nn.sigmoid(cf)
    sc = (cf * sg).astype(BF16)
    zero_s[...] = jnp.broadcast_to(jnp.where(sg[:, 0:128] > 2.0, 1, 0), (CH, 128))
    sc8 = jnp.broadcast_to(sc, (8, D))
    n0 = s1_norm(0)
    await_group(1)
    mod_mm(0, HD)
    mod_mm(D, D + HD)
    ha = [s1_mod(n0, 0, HD)]

    def perm2(t):
        for r in range(0, HD, 128):
            perm_cols(t, r, r + 128)

    def mm2(h, t, cur):
        for r in range(0, HD, 128):
            s1_mm(h[:, r:r + 128], t, cur, None, r, r + 128)

    await_group(2)
    perm2(0)
    mm2(ha[0], 0, sets[0])
    await_group(3)
    perm2(1)
    n1 = s1_norm(1)
    ha.append(s1_mod(n1, 0, HD))
    mm2(ha[0], 1, sets[0])
    s1_mm(ha[1], 0, sets[1], None, 0, HD)
    s1_mm(ha[1], 1, sets[1], None, 0, HD)
    await_group(GI['qk1'])
    perm_cols(0, HD, D)
    mod_mm(HD, D)
    mod_mm(D + HD, 2 * D)
    perm_cols(1, HD, D)
    hb = [s1_mod(n, HD, D) for n in (n0, n1)]
    s1_mm(hb[0], 0, sets[0], None, HD, D)
    s1_mm(hb[0], 1, sets[0], None, HD, D)
    s1_mm(hb[1], 0, sets[1], None, HD, D)
    s1_mm(hb[1], 1, sets[1], None, HD, D)
    h01 = [jnp.concatenate([ha[u], hb[u]], axis=1) for u in range(2)]
    await_group(GI['wv'])
    perm_cols(2)
    wv = perm_wo()
    for c in range(NC):
        hg = rgate(h01[0], wv[c], c)
        sets[0][2][c, HALO:HALO + TM, :] = _dot(hg, wqkv_p[:, 2 * D + c * 128:2 * D + (c + 1) * 128])
    for t in (1, 2):
        for c in range(NC):
            sets[0][t][c, 0:HALO, :] = jnp.broadcast_to(sets[0][t][c, HALO:HALO + 1, :], (HALO, 128))
    seq = []
    s1_mm(h01[1], 2, sets[1], seq)
    s1_halo(sets[0], sets[1])
    s1(2, sets[1], sets[2], seq)
    s2(True, sets[0], o_nxt, make_gate(seq, GP1), ln=3)
    x1_s[0:TM, :] = _dot(o_nxt[...], wo_p[...])
    await_group(GI['m2'])
    seq = []
    jobs = list(range(3 * NC, 5 * NC)) + list(range(2 * NC, 3 * NC)) + list(range(5 * NC, 6 * NC))
    h3 = h1_s[...]
    s1_halo(sets[2], sets[3])
    mm_mod(h3, 0, sets[3], seq, jobs, 2)
    mm_mod(h3, 1, sets[3], seq, jobs, 2)
    s1_mm(h3, 2, sets[3], seq)
    h2x_s[...] = s3(0, None, x1_s[0:TM, :])
    h2_0 = h2x_s[...]
    for k in range(KD):
        if k == KATT:
            s2(False, sets[1], o_cur, make_gate(seq, GP1B))
            h2_s[...] = s3(1, o_cur)
        t = _dot(h2_0, w1_v[:, k * FC:(k + 1) * FC])
        seq.append(t)
        g0_s[:, k * FC:(k + 1) * FC] = act(t)
    await_group(GI['w2'])

    def body(i, carry):
        s4_attn(i, h2_s[...], ring(i + 1), o_cur, i + 3)
        h2_s[...] = s3(i + 1, o_cur)
        s1(None, ring(i), ring(i + 1))
        o_copy(i).start()
        return carry

    lax.fori_loop(1, NB - 3, body, 0)

    seq = []
    s4(5, h2_s[...], seq)
    o_copy(5).start()
    s2(False, ring(6), o_cur, make_gate(seq, GSPAN, wt=False))
    h2_6 = s3(6, o_cur)
    t0 = _dot(h2x_s[...], w1_v[:, KD * FC:F])
    y0 = _dot(g0_s[:, 0:KD * FC], w2_v[0:KD * FC, :])
    y0 = y0 + _dot(act(t0), w2_v[KD * FC:F, :])
    s4_out(0, y0)
    o_copy(0).start()
    st = {}

    def mid(k, g):
        if k == KT7:
            s2(False, ring(7), o_nxt, make_gate([y0[:, :256], y0[:, 256:]] * 1 + seq6, GT7, GT7O, wt=False))
            st['h'] = s3(7, o_nxt)
        return g

    seq6 = []
    s4(6, h2_6, seq6, mid)
    o_copy(6).start()
    s4(7, st['h'], [], last=True)
    for i in range(NB - 1):
        o_copy(i).wait()
    for u in range(NLAST):
        ol_copy(u).wait()


@jax.jit
def pallas_adaLN_cond__sliding_local_dilated__dense_activation_silu__prompt_kernel(
    A_x, A_wqkv, A_wo, B_x, B_w1, B_w2, c, w_mod):
    any_spec = pl.BlockSpec(memory_space=pl.ANY)
    qkv_set = [pltpu.VMEM((TM, D), F32),
               pltpu.VMEM((NC, TM + HALO, 128), F32),
               pltpu.VMEM((NC, TM + HALO, 128), F32)]
    return pl.pallas_call(
        _kernel,
        out_shape=jax.ShapeDtypeStruct((1, S, D), BF16),
        in_specs=[any_spec] * 7,
        out_specs=any_spec,
        scratch_shapes=[
            pltpu.VMEM((S, D), BF16),
            pltpu.VMEM((D, 3 * D), BF16),
            pltpu.VMEM((D, 3 * D), BF16),
            pltpu.VMEM((D, D), BF16),
            pltpu.VMEM((D, D), BF16),
            pltpu.VMEM((D, F), BF16),
            pltpu.VMEM((F, D), BF16),
            pltpu.VMEM((D, 6 * D), BF16),
            pltpu.VMEM((S, D), BF16),
            *[pltpu.VMEM((2,) + t.shape, F32) for t in qkv_set], *qkv_set, *qkv_set,
            pltpu.VMEM((TM, D), BF16),
            pltpu.VMEM((TM, D), BF16),
            pltpu.VMEM((S, D), F32),
            pltpu.VMEM((TM, D), BF16),
            pltpu.VMEM((TM, D), BF16),
            pltpu.VMEM((TM, D), BF16),
            pltpu.VMEM((TM, F), BF16),
            pltpu.VMEM((NC, 128, 128), BF16),
            pltpu.VMEM((8, 6 * D), F32),
            pltpu.VMEM((CH, 128), jnp.int32),
            pltpu.VMEM((1, D), BF16),
            pltpu.VMEM((NC, (H + 1) * PT, 128), F32),
            pltpu.SemaphoreType.DMA((NS,)),
        ],
        compiler_params=pltpu.CompilerParams(vmem_limit_bytes=64 * 1024 * 1024),
    )(A_x, A_wqkv, A_wo, B_w1, B_w2, c, w_mod)
```
